```python
import jax
import jax.numpy as jnp

def _softmax(x, axis=-1):
    return jax.nn.softmax(x, axis=axis)

def _gelu(x):
    return jax.nn.gelu(x, approximate=True)

def _silu(x):
    return jax.nn.silu(x)

def _sigmoid(x):
    return jax.nn.sigmoid(x)

def _layernorm(x, axis=-1, eps=1e-05):
    m = jnp.mean(x, axis=axis, keepdims=True)
    v = jnp.var(x, axis=axis, keepdims=True)
    return (x - m) / jnp.sqrt(v + eps)

def _scatter_add(tgt, idx, src, axis=0):
    return tgt.at[idx].add(src)

def _segment_sum(src, seg, n):
    return jax.ops.segment_sum(src, seg, n)

class _Rng:

    def __init__(self, key):
        self._k = key

    def _next(self):
        self._k, sub = jax.random.split(self._k)
        return sub

    def normal(self, shape):
        return jax.random.normal(self._next(), shape, dtype=jnp.bfloat16)

    def randint(self, lo, hi, shape):
        return jax.random.randint(self._next(), shape, lo, hi, dtype=jnp.int32)

    def uniform(self, shape, lo=0.0, hi=1.0):
        return jax.random.uniform(self._next(), shape, jnp.bfloat16, lo, hi)

    def permutation(self, n):
        return jax.random.permutation(self._next(), n)
kernel_name = 'adaLN_cond__sliding_block_cached__mixer_token_mlp__decode'

def setup_inputs():
    _rng = _Rng(jax.random.key(int.from_bytes(__import__("os").urandom(4), "little")))
    _w = lambda a: (lambda t: t.astype(jnp.bfloat16) if jnp.issubdtype(t.dtype, jnp.floating) else t)(jnp.asarray(a))

    def _A_setup():
        B, Sq, D = (1, 1, 640)
        Hq, Hkv, Sk, Dh = (32, 32, 32768, 192)
        assert Hq % Hkv == 0, (Hq, Hkv)
        return {'x': _w((lambda *s: _rng.normal(s) * 0.05)(B, Sq, D)), 'k_cache': _w((lambda *s: _rng.normal(s) * 0.05)(B, Hkv, Sk, Dh)), 'v_cache': _w((lambda *s: _rng.normal(s) * 0.05)(B, Hkv, Sk, Dh)), 'wq': _w((lambda *s: _rng.normal(s) * 0.05)(D, Hq * Dh) * D ** (-0.5)), 'wo': _w((lambda *s: _rng.normal(s) * 0.05)(Hq * Dh, D) * (Hq * Dh) ** (-0.5))}
    _A_in = _A_setup()

    def _B_setup():
        B, S, D, F = (1, 1, 640, 1536)
        return {'x': _w((lambda *s: _rng.normal(s) * 0.05)(B, S, D)), 'w1': _w((lambda *s: _rng.normal(s) * 0.05)(S, F) * S ** (-0.5)), 'b1': _w((lambda *s: _rng.normal(s) * 0.05)(F) * 0.02), 'w2': _w((lambda *s: _rng.normal(s) * 0.05)(F, S) * F ** (-0.5)), 'b2': _w((lambda *s: _rng.normal(s) * 0.05)(S) * 0.02)}
    _B_in = _B_setup()
    return {'A_x': _A_in['x'], 'A_k_cache': _A_in['k_cache'], 'A_v_cache': _A_in['v_cache'], 'A_wq': _A_in['wq'], 'A_wo': _A_in['wo'], 'B_x': _B_in['x'], 'B_w1': _B_in['w1'], 'B_b1': _B_in['b1'], 'B_w2': _B_in['w2'], 'B_b2': _B_in['b2'], 'c': _w((lambda *s: _rng.normal(s) * 0.05)(1, 640)), 'w_mod': _w((lambda *s: _rng.normal(s) * 0.05)(640, 6 * 640) * 640 ** (-0.5))}

def reference(A_x, A_k_cache, A_v_cache, A_wq, A_wo, B_x, B_w1, B_b1, B_w2, B_b2, c, w_mod):

    def _A_ref(x, k_cache, v_cache, wq, wo):
        B, Sq, D = x.shape
        Hq, Dh = (32, 192)
        Hkv, Sk = (k_cache.shape[1], k_cache.shape[2])
        W = min(4096, max(256, Sk // 4))
        rep = Hq // Hkv
        q = (lambda x, *d: x.transpose(*d))((x @ wq).reshape(B, Sq, Hq, Dh), 0, 2, 1, 3)
        k = jnp.repeat(k_cache[:, :, Sk - W:, :], rep, axis=1)
        v = jnp.repeat(v_cache[:, :, Sk - W:, :], rep, axis=1)
        scores = jnp.einsum('bhqd,bhkd->bhqk', q, k) * Dh ** (-0.5)
        p = _softmax(scores, axis=-1)
        o = jnp.einsum('bhqk,bhkd->bhqd', p, v)
        return (lambda x, *d: x.transpose(*d))(o, 0, 2, 1, 3).reshape(B, Sq, Hq * Dh) @ wo

    def _B_ref(x, w1, b1, w2, b2):
        B, S, D = x.shape
        h = _layernorm(x, axis=-1)
        u = jnp.einsum('bsd,sf->bdf', h, w1) + b1
        u = _gelu(u)
        y = jnp.einsum('bdf,fs->bds', u, w2) + b2
        return (lambda x, *d: x.transpose(*d))(y, 0, 2, 1)
    x = A_x
    mod = (_silu(c) @ w_mod).reshape(c.shape[0], 6, 1, -1)
    sa, ca, ga, sb, cb, gb = (mod[:, 0].copy(), mod[:, 1].copy(), mod[:, 2].copy(), mod[:, 3].copy(), mod[:, 4].copy(), mod[:, 5].copy())
    h = _layernorm(x, axis=-1) * (1 + ca) + sa
    x = x + ga * _A_ref(h, A_k_cache, A_v_cache, A_wq, A_wo)
    h = _layernorm(x, axis=-1) * (1 + cb) + sb
    x = x + gb * _B_ref(h, B_w1, B_b1, B_w2, B_b2)
    return x
```

```python
import functools
import math

import jax
import jax.numpy as jnp
from jax import lax
import jax.experimental.pallas as pl
import jax.experimental.pallas.tpu as pltpu

F32 = jnp.float32
BF16 = jnp.bfloat16

HQ = 32
DH = 192
PAIR = 2 * DH
NPAIR = HQ // 2
EPS = 1e-5
GELU_C = math.sqrt(2.0 / math.pi)
GELU_A = 0.044715

S_SMALL, S_WMOD, S_WQ, S_GB = 0, 1, 2, 3
S_K, S_V, S_WO = 4, 6, 8
S_TAIL = 10
TAIL_CHUNKS = (1024, 1024, 512, 512, 512, 256, 256)
N_SEMS = S_TAIL + len(TAIL_CHUNKS)


def _layernorm(x):
    m = jnp.mean(x, axis=-1, keepdims=True)
    xc = x - m
    v = jnp.mean(xc * xc, axis=-1, keepdims=True)
    return xc * lax.rsqrt(v + EPS)


def _kernel(x_hbm, k_hbm, v_hbm, wq_hbm, wo_hbm, w1_hbm, b1_hbm, w2_hbm, b2_hbm,
            c_hbm, wm_hbm, o_ref,
            x_v, c_v, w1_v, b1_v, w2_v, b2_v, wm_v, gb_v, wq_v, wo_v, k_v, v_v,
            q_v, p_v, w1c, b1c, w2c, sems, *, D, F, SK, W):
    col0 = SK - W
    ncb = W // 128

    def wait_all(buf, sem):
        pltpu.make_async_copy(buf, buf, sem).wait()

    small = [(x_hbm, x_v), (c_hbm, c_v), (w1_hbm, w1_v), (b1_hbm, b1_v),
             (w2_hbm, w2_v), (b2_hbm, b2_v)]

    def kv_piece(src, dst, pair, slot, half, cb, sem, prio):
        c = cb * 128
        if not isinstance(cb, int):
            c = pl.multiple_of(c, 128)
        pltpu.make_async_copy(
            src.at[pair, pl.ds(half * DH, DH), pl.ds(col0 + c, 128)],
            dst.at[slot, pl.ds(half * DH, DH), pl.ds(c, 128)],
            sem).start(priority=prio)

    def issue_wo(pair, slot):
        for j in range(PAIR // 32):
            pltpu.make_async_copy(
                wo_hbm.at[pair, pl.ds(j * 32, 32), :],
                wo_v.at[slot, pl.ds(j * 32, 32), :],
                sems.at[S_WO + slot]).start(priority=j % 2)

    def issue_k_only(pair, slot):
        def body(cb, carry):
            kv_piece(k_hbm, k_v, pair, slot, 0, cb, sems.at[S_K + slot], 0)
            kv_piece(k_hbm, k_v, pair, slot, 1, cb, sems.at[S_K + slot], 1)
            return carry
        lax.fori_loop(0, ncb, body, 0, unroll=4)

    def issue_kv(s):
        ks = s % 2
        vs = (s - 1) % 2
        issue_wo(s - 1, vs)
        for half in range(2):
            def body(cb, carry):
                kv_piece(k_hbm, k_v, s, ks, half, cb, sems.at[S_K + ks], 0)
                kv_piece(v_hbm, v_v, s - 1, vs, half, cb, sems.at[S_V + vs], 1)
                return carry
            lax.fori_loop(0, ncb, body, 0, unroll=4)

    def issue_tail():
        pair = NPAIR - 1
        vs = pair % 2
        issue_wo(pair, vs)
        cb = 0
        for ci, cw in enumerate(TAIL_CHUNKS):
            for _ in range(cw // 128):
                kv_piece(v_hbm, v_v, pair, vs, 0, cb, sems.at[S_TAIL + ci], 0)
                kv_piece(v_hbm, v_v, pair, vs, 1, cb, sems.at[S_TAIL + ci], 1)
                cb += 1
        for j in range(D // 32):
            pltpu.make_async_copy(
                wm_hbm.at[pl.ds(j * 32, 32), pl.ds(5 * D, D)],
                gb_v.at[pl.ds(j * 32, 32), :],
                sems.at[S_GB]).start(priority=j % 2)

    for src, dst in small:
        pltpu.make_async_copy(src, dst, sems.at[S_SMALL]).start()

    def wm_body(j, carry):
        r = pl.multiple_of(j * 32, 32)
        for sec in range(5):
            pltpu.make_async_copy(
                wm_hbm.at[pl.ds(r, 32), pl.ds(sec * D, D)],
                wm_v.at[pl.ds(r, 32), pl.ds(sec * D, D)],
                sems.at[S_WMOD]).start(priority=sec % 2)
        return carry
    lax.fori_loop(0, D // 32, wm_body, 0)

    NQ = HQ * DH

    def wq_body(j, carry):
        r = pl.multiple_of(j * 16, 16)
        for sec in range(4):
            pltpu.make_async_copy(
                wq_hbm.at[pl.ds(r, 16), pl.ds(sec * (NQ // 4), NQ // 4)],
                wq_v.at[pl.ds(r, 16), pl.ds(sec * (NQ // 4), NQ // 4)],
                sems.at[S_WQ]).start(priority=sec % 2)
        return carry
    lax.fori_loop(0, D // 16, wq_body, 0)

    for src, dst in small:
        pltpu.make_async_copy(src, dst, sems.at[S_SMALL]).wait()
    wait_all(wm_v, sems.at[S_WMOD])

    x = x_v[...].astype(F32)
    cc = c_v[...].astype(F32)
    sc = cc * jax.nn.sigmoid(cc)
    sc8 = jnp.broadcast_to(sc, (8, D)).astype(BF16)
    mod = jnp.dot(sc8, wm_v[...], preferred_element_type=F32)[0:1]
    sa, ca, ga = mod[:, 0:D], mod[:, D:2 * D], mod[:, 2 * D:3 * D]
    sb, cb_ = mod[:, 3 * D:4 * D], mod[:, 4 * D:5 * D]
    h = _layernorm(x) * (1.0 + ca) + sa
    h8 = jnp.broadcast_to(h, (8, D)).astype(BF16)

    issue_k_only(0, 0)

    eye = (lax.broadcasted_iota(jnp.int32, (128, 128), 0)
           == lax.broadcasted_iota(jnp.int32, (128, 128), 1))
    ones = jnp.ones((128, 128), BF16)
    w1r = w1_v[...].astype(F32)
    w2r = w2_v[...].astype(F32)
    b1r = b1_v[...].astype(F32)
    lin_a = jnp.zeros((1, 128), F32)
    lin_b = jnp.zeros((1, 128), F32)
    for j in range(F // 128):
        r1 = w1r[:, j * 128:(j + 1) * 128]
        rb = b1r[j:j + 1, :]
        r2 = w2r[:, j * 128:(j + 1) * 128]
        for row, dst, scale in ((r1, w1c, 1.0), (rb, b1c, 1.0), (r2, w2c, 0.5)):
            diag = jnp.where(eye, jnp.broadcast_to(row, (128, 128)), 0.0).astype(BF16)
            col = jnp.dot(diag, ones, preferred_element_type=F32)
            dst[j * 128:(j + 1) * 128, :] = col * scale
        lin_a = lin_a + r1 * r2
        lin_b = lin_b + rb * r2
    lin_a = 0.5 * jnp.sum(lin_a, axis=-1, keepdims=True)
    lin_b = 0.5 * jnp.sum(lin_b, axis=-1, keepdims=True) + b2_v[...].astype(F32)

    issue_kv(1)

    wait_all(wq_v, sems.at[S_WQ])
    row = lax.broadcasted_iota(jnp.int32, (8, PAIR), 0)
    lane = lax.broadcasted_iota(jnp.int32, (8, PAIR), 1)
    own = (lane >= DH) == (row == 1)
    q_all = jnp.dot(h8, wq_v[...], preferred_element_type=F32)
    for p in range(NPAIR):
        q_v[p] = jnp.where(own, q_all[:, p * PAIR:(p + 1) * PAIR], 0.0).astype(BF16)

    scale = DH ** -0.5

    def scores(pair, slot):
        s = jnp.dot(q_v[pair], k_v[slot], preferred_element_type=F32) * scale
        m = jnp.max(s, axis=-1, keepdims=True)
        e = jnp.exp(s - m)
        l = jnp.sum(e, axis=-1, keepdims=True)
        p_v[...] = e.astype(BF16)
        return 1.0 / l

    nt = (((1,), (1,)), ((), ()))

    def project(o, inv_l, slot):
        o = jnp.where(own & (row < 2), o * inv_l, 0.0).astype(BF16)
        return jnp.dot(o, wo_v[slot], preferred_element_type=F32)

    wait_all(k_v.at[0], sems.at[S_K])
    inv_l0 = scores(0, 0)

    def stage(s, carry, last):
        acc, inv_l = carry
        if last:
            issue_tail()
        else:
            issue_kv(s + 1)
        ks = s % 2
        vs = (s - 1) % 2
        wait_all(v_v.at[vs], sems.at[S_V + vs])
        wait_all(wo_v.at[vs], sems.at[S_WO + vs])
        o = lax.dot_general(p_v[...], v_v[vs], nt, preferred_element_type=F32)
        acc = acc + project(o, inv_l, vs)
        wait_all(k_v.at[ks], sems.at[S_K + ks])
        inv_l = scores(s, ks)
        return acc, inv_l

    carry = (jnp.zeros((8, D), F32), inv_l0)
    carry = lax.fori_loop(1, NPAIR - 1, functools.partial(stage, last=False), carry)
    acc, inv_l = stage(NPAIR - 1, carry, True)

    vs = (NPAIR - 1) % 2
    wait_all(wo_v.at[vs], sems.at[S_WO + vs])
    o = jnp.zeros((8, PAIR), F32)
    c0 = 0
    for ci, cw in enumerate(TAIL_CHUNKS):
        wait_all(v_v.at[vs, :, pl.ds(c0, cw)], sems.at[S_TAIL + ci])
        o = o + lax.dot_general(p_v[:, c0:c0 + cw], v_v[vs, :, c0:c0 + cw], nt,
                                preferred_element_type=F32)
        c0 += cw
    acc = acc + project(o, inv_l, vs)
    attn = acc[0:1] + acc[1:2]

    x1 = x + ga * attn
    g = _layernorm(x1) * (1.0 + cb_) + sb
    hm = _layernorm(g)
    hb = jnp.broadcast_to(hm, (8, D))

    def mlp_body(i, y):
        r = pl.multiple_of(i * 8, 8)
        w1 = jnp.concatenate([w1c[pl.ds(r, 8), :]] * (D // 128), axis=1)
        b1 = jnp.concatenate([b1c[pl.ds(r, 8), :]] * (D // 128), axis=1)
        w2 = jnp.concatenate([w2c[pl.ds(r, 8), :]] * (D // 128), axis=1)
        u = hb * w1 + b1
        z = u * (u * u * (GELU_C * GELU_A) + GELU_C)
        return y + (u * w2) * jnp.tanh(z)

    y = lax.fori_loop(0, F // 8, mlp_body, jnp.zeros((8, D), F32), unroll=8)
    y = jnp.sum(y, axis=0, keepdims=True) + hm * lin_a + lin_b

    wait_all(gb_v, sems.at[S_GB])
    gb = jnp.dot(sc8, gb_v[...], preferred_element_type=F32)[0:1]
    o_ref[...] = (x1 + gb * y).astype(o_ref.dtype)


@jax.jit
def pallas_adaLN_cond__sliding_block_cached__mixer_token_mlp__decode_kernel(
    A_x: jax.Array,
    A_k_cache: jax.Array,
    A_v_cache: jax.Array,
    A_wq: jax.Array,
    A_wo: jax.Array,
    B_x: jax.Array,
    B_w1: jax.Array,
    B_b1: jax.Array,
    B_w2: jax.Array,
    B_b2: jax.Array,
    c: jax.Array,
    w_mod: jax.Array,
):
    B, SQ, D = A_x.shape
    _, HKV, SK, dh = A_k_cache.shape
    assert B == 1 and SQ == 1 and HKV == HQ and dh == DH
    S, F = B_w1.shape
    assert S == 1
    W = min(4096, max(256, SK // 4))
    assert sum(TAIL_CHUNKS) == W

    kt = jnp.swapaxes(A_k_cache, 2, 3).reshape(NPAIR, PAIR, SK)
    vt = jnp.swapaxes(A_v_cache, 2, 3).reshape(NPAIR, PAIR, SK)
    args = (
        A_x.reshape(1, D), kt, vt, A_wq, A_wo.reshape(NPAIR, PAIR, D),
        B_w1, B_b1.reshape(F // 128, 128), B_w2.reshape(1, F), B_b2.reshape(1, 1),
        c, w_mod,
    )
    out = pl.pallas_call(
        functools.partial(_kernel, D=D, F=F, SK=SK, W=W),
        out_shape=jax.ShapeDtypeStruct((1, D), A_x.dtype),
        in_specs=[pl.BlockSpec(memory_space=pl.ANY)] * len(args),
        out_specs=pl.BlockSpec(memory_space=pltpu.VMEM),
        scratch_shapes=[
            pltpu.VMEM((1, D), BF16),
            pltpu.VMEM((1, D), BF16),
            pltpu.VMEM((1, F), BF16),
            pltpu.VMEM((F // 128, 128), BF16),
            pltpu.VMEM((1, F), BF16),
            pltpu.VMEM((1, 1), BF16),
            pltpu.VMEM((D, 5 * D), BF16),
            pltpu.VMEM((D, D), BF16),
            pltpu.VMEM((D, HQ * DH), BF16),
            pltpu.VMEM((2, PAIR, D), BF16),
            pltpu.VMEM((2, PAIR, W), BF16),
            pltpu.VMEM((2, PAIR, W), BF16),
            pltpu.VMEM((NPAIR, 8, PAIR), BF16),
            pltpu.VMEM((8, W), BF16),
            pltpu.VMEM((F, 128), F32),
            pltpu.VMEM((F, 128), F32),
            pltpu.VMEM((F, 128), F32),
            pltpu.SemaphoreType.DMA((N_SEMS,)),
        ],
        compiler_params=pltpu.CompilerParams(vmem_limit_bytes=64 * 1024 * 1024),
    )(*args)
    return out.reshape(B, SQ, D)
```

```python
import contextlib
import functools
import math

import jax
import jax.numpy as jnp
from jax import lax
import jax.experimental.pallas as pl
import jax.experimental.pallas.tpu as pltpu

F32 = jnp.float32
BF16 = jnp.bfloat16

HQ = 32
DH = 192
PAIR = 2 * DH
NPAIR = HQ // 2
EPS = 1e-5
GELU_C = math.sqrt(2.0 / math.pi)
GELU_A = 0.044715
GELU_S = (GELU_C * GELU_A) ** (1.0 / 3.0)
GELU_K = GELU_C / GELU_S

TAIL_V = (2048, 1024, 512, 512)
LATE_WO = PAIR
TAIL_WO = (128, 128, 64, 64)
GB_MXU = 384
GB_AT = 11
MOVE = 2
COL_SPLIT = 64
GB_R = 16
LEAD = 32
WM_G = 4
WQ_G, WQ_C = 5, 512
WO_G = 3

S_SMALL, S_WMOD, S_WQ, S_WO = 0, 1, 2, 3
S_K, S_V = 4, 6
S_TV, S_TO, S_GB = 8, 16, 24
N_SEMS = 32
SKIP_ATT = False
SKIP_MLP = False
NOBC = True
SCOPES = False


def _scope(name):
    return jax.named_scope(name) if SCOPES else contextlib.nullcontext()


def _layernorm(x):
    m = jnp.mean(x, axis=-1, keepdims=True)
    xc = x - m
    v = jnp.mean(xc * xc, axis=-1, keepdims=True)
    return xc * lax.rsqrt(v + EPS)


def _chunk_of(pos, chunks):
    c0 = 0
    for ci, cw in enumerate(chunks):
        c0 += cw
        if pos < c0:
            return ci


def _sublane_allsum(x):
    x = x + pltpu.roll(x, 4, 0)
    x = x + pltpu.roll(x, 2, 0)
    return x + pltpu.roll(x, 1, 0)


def _kernel(x_hbm, k_hbm, v_hbm, wq_hbm, wo_hbm, w1_hbm, b1_hbm, w2_hbm, b2_hbm,
            c_hbm, wm_hbm, wm2_hbm, o_ref,
            x_v, c_v, w1_v, b1_v, w2_v, b2_v, wm_v, gb_v, wq_v, wo_v, k_v, v_v,
            q_v, p_v, o_v, t_v, th_v, w1c, b1c, scc, occ, lhs_v, sems, *, D, F, SK, W):
    col0 = SK - W
    ncb = W // 128
    NQ = HQ * DH
    nd = D // 128

    def wait_all(buf, sem, name='w'):
        with _scope('wait_' + name):
            pltpu.make_async_copy(buf, buf, sem).wait()

    small = [(x_hbm, x_v), (c_hbm, c_v), (w1_hbm, w1_v), (b1_hbm, b1_v),
             (w2_hbm, w2_v), (b2_hbm, b2_v)]

    def kv_piece(is_v, pair, half, cb, sem=None):
        src, dst, s0 = (v_hbm, v_v, S_V) if is_v else (k_hbm, k_v, S_K)
        slot = pair % 2
        c = cb * 128
        if not isinstance(cb, int):
            c = pl.multiple_of(c, 128)
        return pltpu.make_async_copy(
            src.at[pair, pl.ds(half * DH, DH), pl.ds(col0 + c, 128)],
            dst.at[slot, pl.ds(half * DH, DH), pl.ds(c, 128)],
            sems.at[s0 + slot] if sem is None else sem)

    def last_v_piece(half, cb):
        return kv_piece(True, NPAIR - 1, half, cb, sems.at[S_TV + _chunk_of(cb * 128, TAIL_V)])

    def wm_piece(r, sec):
        return pltpu.make_async_copy(
            wm_hbm.at[:, pl.ds(r, 8), pl.ds(sec * D, D)],
            wm_v.at[:, pl.ds(r, 8), pl.ds(sec * D, D)], sems.at[S_WMOD])

    def wq_piece(r, c):
        return pltpu.make_async_copy(
            wq_hbm.at[:, pl.ds(r, 8), pl.ds(c, WQ_C)], wq_v.at[:, pl.ds(r, 8), pl.ds(c, WQ_C)],
            sems.at[S_WQ])

    nblk = NQ // WO_G // 128
    b_late = nblk - 2 * (PAIR // 128)

    def wo_piece(b, r):
        g = WO_G - 1 if b_late <= b < b_late + PAIR // 128 else WO_G
        return pltpu.make_async_copy(
            wo_hbm.at[pl.ds(0, g), b, pl.ds(r, 8), :], wo_v.at[pl.ds(0, g), b, pl.ds(r, 8), :],
            sems.at[S_WO])

    def late_wo_piece(r):
        b = b_late + r // 128
        return pltpu.make_async_copy(
            wo_hbm.at[WO_G - 1, b, pl.ds(r % 128, 32), :], wo_v.at[WO_G - 1, b, pl.ds(r % 128, 32), :],
            sems.at[S_TO + _chunk_of(r, TAIL_WO)])

    def gb_piece(r):
        return pltpu.make_async_copy(
            wm2_hbm.at[pl.ds(r, GB_R), pl.ds(5 * D, D)], gb_v.at[pl.ds(r, GB_R), :],
            sems.at[S_GB])

    P = functools.partial
    wm_p = [P(wm_piece, r, s) for r in range(0, D // WM_G, 8) for s in range(5)]
    wq_p = [P(wq_piece, r, c) for r in range(0, D // WQ_G, 8) for c in range(0, NQ, WQ_C)]
    wo_p = [P(wo_piece, b, r) for b in range(NQ // WO_G // 128) for r in range(0, 128, 8)]
    lw_p = [P(late_wo_piece, r) for r in range(0, LATE_WO, 32)]
    gb_p = [P(gb_piece, r) for r in range(0, D, GB_R)]

    def halves(lst):
        h = len(lst) // 2
        return lst[:h], lst[h:]

    def merge(a, b):
        out = []
        for i in range(max(len(a), len(b))):
            if i < len(a):
                out.append((a[i], 0))
            if i < len(b):
                out.append((b[i], 1))
        return out

    wmA, wmB = halves(wm_p)
    wqA, wqB = halves(wq_p)
    woA, woB = halves(wo_p)
    seqA = wmA + wqA + woA
    seqB = wmB + wqB + woB + [P(kv_piece, False, 0, 1, cb) for cb in range(ncb)]
    order = [(f, 1) for f in seqB[:LEAD]] + merge(seqA, seqB[LEAD:])
    cut1 = LEAD + 2 * (len(wmA) + 28)
    cut2 = LEAD + 2 * (len(wmA) + len(wqA) + 28)

    def issue(lst, name='issue'):
        with _scope(name):
            for f, prio in lst:
                f().start(priority=prio)

    def issue_batch(is_v, pair):
        nv, npair = (False, pair + 1) if is_v else (True, pair)

        def body(cb, carry):
            kv_piece(is_v, pair, 0, cb).start(priority=0)
            kv_piece(nv, npair, 1, cb).start(priority=1)
            return carry
        with _scope('issue'):
            lax.fori_loop(0, ncb, body, 0, unroll=4)

    for src, dst in small:
        pltpu.make_async_copy(src, dst, sems.at[S_SMALL]).start()
    issue(order[:cut1])

    for src, dst in small:
        pltpu.make_async_copy(src, dst, sems.at[S_SMALL]).wait()
    wait_all(wm_v, sems.at[S_WMOD], 'wm')

    x = jnp.broadcast_to(x_v[...].astype(F32), (8, D))
    cc = c_v[...].astype(F32)
    sc = (cc * jax.nn.sigmoid(cc)).astype(BF16)
    sc8 = jnp.broadcast_to(sc.astype(F32), (8, D)).astype(BF16)
    mod = jnp.dot(sc8, wm_v[...].reshape(D, 5 * D), preferred_element_type=F32)
    sa, ca, ga, sb, cb1 = (mod[:, i * D:(i + 1) * D] for i in range(5))
    mean = lambda t: jnp.mean(t, axis=-1, keepdims=True)
    A = 1.0 + cb1
    Bc = sb - mean(sb)
    A2, AB = A * A, A * Bc
    eA, eA2, eAB, eB2 = mean(A), mean(A2), mean(AB), mean(Bc * Bc)
    h8 = (_layernorm(x) * (1.0 + ca) + sa).astype(BF16)

    eye = (lax.broadcasted_iota(jnp.int32, (128, 128), 0)
           == lax.broadcasted_iota(jnp.int32, (128, 128), 1))
    ones = jnp.ones((128, 128), BF16)

    def column(rowvec, split=128):
        diag = jnp.where(eye, jnp.broadcast_to(rowvec, (128, 128)), 0.0).astype(BF16)
        return jnp.concatenate(
            [jnp.dot(diag[r:r + split], ones, preferred_element_type=F32)
             for r in range(0, 128, split)], axis=0)

    scf = sc.astype(F32)
    for j in range(GB_MXU // 128, nd):
        scc[j * 128:(j + 1) * 128, :] = column(scf[:, j * 128:(j + 1) * 128])

    w1r = w1_v[...].astype(F32)
    w2r = w2_v[...].astype(F32)
    b1r = b1_v[...].astype(F32)
    row128 = lax.broadcasted_iota(jnp.int32, (8, 128), 0)
    lin = jnp.zeros((8, 128), F32)
    for j in range(F // 128):
        r1 = w1r[:, j * 128:(j + 1) * 128]
        rb = b1r[j:j + 1, :]
        r2 = w2r[:, j * 128:(j + 1) * 128]
        w1c[j * 128:(j + 1) * 128, :] = column(r1) * GELU_S
        b1c[j * 128:(j + 1) * 128, :] = column(rb) * GELU_S
        t = jnp.where(row128 < 4, r1, rb) * (0.5 * r2)
        hi = t.astype(BF16).astype(F32)
        lo = (t - hi).astype(BF16).astype(F32)
        lhs_v[:, j * 128:(j + 1) * 128] = jnp.where(
            row128 % 4 == 0, hi, jnp.where(row128 % 4 == 1, lo, 0.0))
        lin = lin + t
    lin = jnp.sum(lin, axis=-1, keepdims=True)
    lin = lin + jnp.where(lax.broadcasted_iota(jnp.int32, (8, 1), 0) < 4, 0.0,
                          b2_v[...].astype(F32))
    rowD = lax.broadcasted_iota(jnp.int32, (8, D), 0)
    lin = jnp.where(rowD % 4 == 0, jnp.broadcast_to(lin, (8, D)), 0.0)

    issue(order[cut1:cut2])

    wait_all(wq_v, sems.at[S_WQ], 'wq')
    row = lax.broadcasted_iota(jnp.int32, (8, PAIR), 0)
    lane = lax.broadcasted_iota(jnp.int32, (8, PAIR), 1)
    own = (lane >= DH) == (row % 2 == 1)
    q_all = jnp.dot(h8, wq_v[...].reshape(D, NQ), preferred_element_type=F32)
    for p in range(NPAIR):
        q_v[p] = jnp.where(own, q_all[:, p * PAIR:(p + 1) * PAIR], 0.0).astype(BF16)

    issue(order[cut2:])
    issue_batch(False, 0)
    wait_all(wo_v.at[pl.ds(0, WO_G - 1)], sems.at[S_WO], 'wo')
    wait_all(wo_v.at[WO_G - 1, pl.ds(0, b_late)], sems.at[S_WO], 'wo')
    wait_all(wo_v.at[WO_G - 1, pl.ds(b_late + PAIR // 128, PAIR // 128)], sems.at[S_WO], 'wo')

    scale = DH ** -0.5

    def scores(pair):
        slot = pair % 2
        wait_all(k_v.at[slot], sems.at[S_K + slot], 'k')
        if SKIP_ATT:
            p_v[...] = jnp.zeros(p_v.shape, BF16)
            return jnp.ones((8, 1), F32)
        s = jnp.dot(q_v[pair], k_v[slot], preferred_element_type=F32) * scale
        m = jnp.max(s, axis=-1, keepdims=True)
        e = jnp.exp(s - m)
        l = jnp.sum(e, axis=-1, keepdims=True)
        p_v[...] = e.astype(BF16)
        return 1.0 / l

    nt = (((1,), (1,)), ((), ()))

    def project(o, inv_l, pair):
        o = jnp.where(own, o * inv_l, 0.0).astype(BF16)
        r = None
        for i in range(PAIR // 128):
            j = pair * (PAIR // 128) + i
            t = jnp.dot(o[:, i * 128:(i + 1) * 128], wo_v[j // nblk, j % nblk],
                        preferred_element_type=F32)
            r = t if r is None else r + t
        return r

    def values(s, acc, inv_l):
        slot = s % 2
        wait_all(v_v.at[slot], sems.at[S_V + slot], 'v')
        if SKIP_ATT:
            return acc
        o = lax.dot_general(p_v[...], v_v[slot], nt, preferred_element_type=F32)
        return acc + project(o, inv_l, s)

    def stage(s, acc):
        issue_batch(True, s)
        inv_l = scores(s)
        issue_batch(False, s + 1)
        return values(s, acc, inv_l)

    acc = lax.fori_loop(0, NPAIR - 2, stage, jnp.zeros((8, D), F32))

    last = NPAIR - 1
    issue_batch(True, last - 1)
    inv_l = scores(last - 1)
    issue(merge([P(kv_piece, False, last, 0, cb) for cb in range(ncb)],
                [P(last_v_piece, 1, cb) for cb in range(ncb)]))
    wait_all(v_v.at[(last - 1) % 2], sems.at[S_V + (last - 1) % 2], 'v')
    o = lax.dot_general(p_v[...], v_v[(last - 1) % 2], nt, preferred_element_type=F32)
    o = jnp.where(own, o * inv_l, 0.0)
    o = o + pltpu.roll(o, 1, 0)
    for i in range(PAIR // 128):
        occ[i * 128:(i + 1) * 128, :] = column(o[0:1, i * 128:(i + 1) * 128])

    vA = [P(last_v_piece, 0, cb) for cb in range(ncb)]
    k = ncb - 2 * MOVE
    issue(merge(vA[:k] + vA[k::2] + lw_p[0::2], vA[k + 1::2] + lw_p[1::2] + gb_p))
    inv_l = scores(last)
    xc = x + ga * (acc + pltpu.roll(acc, 1, 0))
    shift = mean(xc)
    xc = xc - shift
    vs = last % 2
    c0 = 0
    for ci, cw in enumerate(TAIL_V):
        wait_all(v_v.at[vs, :, pl.ds(c0, cw)], sems.at[S_TV + ci], 'tv%d' % ci)
        if not SKIP_MLP:
            t = lax.dot_general(p_v[:, c0:c0 + cw], v_v[vs, :, c0:c0 + cw], nt,
                                preferred_element_type=F32)
            if ci > 0:
                t = t + o_v[...]
            if ci < len(TAIL_V) - 1:
                o_v[...] = t
        c0 += cw

    def late_rows(ci):
        r0, n = sum(TAIL_WO[:ci]), TAIL_WO[ci]
        assert r0 % 128 + n <= 128
        return wo_v.at[WO_G - 1, b_late + r0 // 128, pl.ds(r0 % 128, n)], r0, n

    if SKIP_MLP:
        for ci in range(len(TAIL_WO)):
            wait_all(late_rows(ci)[0], sems.at[S_TO + ci], 'to%d' % ci)
        wait_all(gb_v, sems.at[S_GB], 'gb')
        o_ref[...] = (xc + A2 + AB + eA + eA2 + eAB + eB2 + lin)[0:1].astype(o_ref.dtype)
        return

    def vpu_matvec(w, col, part=None):
        for r in range(0, w.shape[0], 16):
            prod = w[r:r + 16, :].astype(F32) * jnp.concatenate([col[r:r + 16, :]] * nd, axis=1)
            part = prod if part is None else part + prod
        return part

    t = project(t, inv_l, last)
    xc = xc + ga * (t + pltpu.roll(t, 1, 0))
    part = None
    for ci in range(len(TAIL_WO)):
        rows, r0, n = late_rows(ci)
        wait_all(rows, sems.at[S_TO + ci], 'to%d' % ci)
        part = vpu_matvec(rows, occ.at[pl.ds(r0, n)], part)
    xc = xc + ga * _sublane_allsum(part[:8] + part[8:])
    x1 = xc + shift

    xa = xc * A
    d1, e2 = mean(xc), mean(xc * xc)
    exa, exa2, exaa, exab = mean(xa), mean(xa * xa), mean(xc * A2), mean(xc * AB)
    r1 = lax.rsqrt(jnp.maximum(e2 - d1 * d1, 0.0) + EPS)
    mu = exa - d1 * eA
    p2 = exa2 - d1 * (2.0 * exaa - d1 * eA2) - mu * mu
    p1 = 2.0 * (exab - d1 * eAB)
    r2 = lax.rsqrt(jnp.maximum((p2 * r1 + p1) * r1 + eB2, 0.0) + EPS)
    hm = ((xa - d1 * A - mu) * r1 + Bc) * r2

    def last_gate():
        wait_all(gb_v, sems.at[S_GB], 'gb')
        gate = jnp.dot(sc8[:, :GB_MXU], gb_v[:GB_MXU, :], preferred_element_type=F32)
        if GB_MXU < D:
            t_v[...] = gate
            vp = vpu_matvec(gb_v.at[pl.ds(GB_MXU, D - GB_MXU)], scc.at[pl.ds(GB_MXU, D - GB_MXU)])
            gate = t_v[...] + _sublane_allsum(vp[:8] + vp[8:])
        return gate

    hb = jnp.concatenate([hm] * 16, axis=0)
    R = lin
    for j in range(F // 128):
        if j == GB_AT:
            gb = last_gate()
        w1 = jnp.concatenate([w1c[j * 128:(j + 1) * 128, :]] * nd, axis=1)
        b1 = jnp.concatenate([b1c[j * 128:(j + 1) * 128, :]] * nd, axis=1)
        s = hb * w1 + b1
        th = jnp.tanh(s * (s * s + GELU_K))
        R = R + jnp.dot(lhs_v[:, j * 128:(j + 1) * 128], th, preferred_element_type=F32)
    if GB_AT == F // 128:
        gb = last_gate()
    R = R + pltpu.roll(R, 7, 0)
    y = hm * R + pltpu.roll(R, 4, 0)
    o_ref[...] = (x1 + gb * y)[0:1].astype(o_ref.dtype)


@jax.jit
def pallas_adaLN_cond__sliding_block_cached__mixer_token_mlp__decode_kernel(
    A_x: jax.Array,
    A_k_cache: jax.Array,
    A_v_cache: jax.Array,
    A_wq: jax.Array,
    A_wo: jax.Array,
    B_x: jax.Array,
    B_w1: jax.Array,
    B_b1: jax.Array,
    B_w2: jax.Array,
    B_b2: jax.Array,
    c: jax.Array,
    w_mod: jax.Array,
):
    B, SQ, D = A_x.shape
    _, HKV, SK, dh = A_k_cache.shape
    assert B == 1 and SQ == 1 and HKV == HQ and dh == DH
    S, F = B_w1.shape
    assert S == 1
    W = min(4096, max(256, SK // 4))
    assert sum(TAIL_V) == W and sum(TAIL_WO) == LATE_WO
    NQ = HQ * DH

    kt = jnp.swapaxes(A_k_cache, 2, 3).reshape(NPAIR, PAIR, SK)
    vt = jnp.swapaxes(A_v_cache, 2, 3).reshape(NPAIR, PAIR, SK)
    args = (
        A_x.reshape(1, D), kt, vt, A_wq.reshape(WQ_G, D // WQ_G, NQ),
        A_wo.reshape(WO_G, NQ // WO_G // 128, 128, D),
        B_w1, B_b1.reshape(F // 128, 128), B_w2.reshape(1, F), B_b2.reshape(1, 1),
        c, w_mod.reshape(WM_G, D // WM_G, 6 * D), w_mod,
    )
    out = pl.pallas_call(
        functools.partial(_kernel, D=D, F=F, SK=SK, W=W),
        out_shape=jax.ShapeDtypeStruct((1, D), A_x.dtype),
        in_specs=[pl.BlockSpec(memory_space=pl.ANY)] * len(args),
        out_specs=pl.BlockSpec(memory_space=pltpu.VMEM),
        scratch_shapes=[
            pltpu.VMEM((1, D), BF16),
            pltpu.VMEM((1, D), BF16),
            pltpu.VMEM((1, F), BF16),
            pltpu.VMEM((F // 128, 128), BF16),
            pltpu.VMEM((1, F), BF16),
            pltpu.VMEM((1, 1), BF16),
            pltpu.VMEM((WM_G, D // WM_G, 5 * D), BF16),
            pltpu.VMEM((D, D), BF16),
            pltpu.VMEM((WQ_G, D // WQ_G, NQ), BF16),
            pltpu.VMEM((WO_G, NQ // WO_G // 128, 128, D), BF16),
            pltpu.VMEM((2, PAIR, W), BF16),
            pltpu.VMEM((2, PAIR, W), BF16),
            pltpu.VMEM((NPAIR, 8, PAIR), BF16),
            pltpu.VMEM((8, W), BF16),
            pltpu.VMEM((8, PAIR), F32),
            pltpu.VMEM((8, D), F32),
            pltpu.VMEM((128, D), F32),
            pltpu.VMEM((F, 128), F32),
            pltpu.VMEM((F, 128), F32),
            pltpu.VMEM((D, 128), F32),
            pltpu.VMEM((PAIR, 128), F32),
            pltpu.VMEM((8, F), F32),
            pltpu.SemaphoreType.DMA((N_SEMS,)),
        ],
        compiler_params=pltpu.CompilerParams(vmem_limit_bytes=64 * 1024 * 1024,
                                             disable_bounds_checks=NOBC),
    )(*args)
    return out.reshape(B, SQ, D)
```

```python
import functools
import math

import jax
import jax.numpy as jnp
from jax import lax
import jax.experimental.pallas as pl
import jax.experimental.pallas.tpu as pltpu

F32 = jnp.float32
BF16 = jnp.bfloat16

HQ = 32
DH = 192
PAIR = 2 * DH
NPAIR = HQ // 2
PB = PAIR // 128
EPS = 1e-5
GELU_C = math.sqrt(2.0 / math.pi)
GELU_A = 0.044715
GELU_S = (GELU_C * GELU_A) ** (1.0 / 3.0)
GELU_K = GELU_C / GELU_S

LEAD = 32
FIFO = 28
WM_G = 4
WQ_G, WQ_C = 5, 512
WO_G = 3
MOVE = 3
TAIL_V = (2048, 1024, 512, 512)
TAIL_WO = (128, 128, 64, 64)
GATE_MXU = 384
GATE_AT = 8

S_SMALL, S_WM, S_WQ = 0, 1, 2
S_WO = 3
S_K, S_V = 6, 8
S_TV = 10
S_TO = S_TV + len(TAIL_V)
S_GB = S_TO + len(TAIL_WO)
N_SEMS = S_GB + 2


def _mean(t):
    return jnp.mean(t, axis=-1, keepdims=True)


def _chunk_of(pos, chunks):
    end = 0
    for ci, n in enumerate(chunks):
        end += n
        if pos < end:
            return ci
    raise ValueError(pos)


def _sublane_allsum(t):
    t = t + pltpu.roll(t, 4, 0)
    t = t + pltpu.roll(t, 2, 0)
    return t + pltpu.roll(t, 1, 0)


def _merge(a, b):
    out = []
    for i in range(max(len(a), len(b))):
        if i < len(a):
            out.append((a[i], 0))
        if i < len(b):
            out.append((b[i], 1))
    return out


def _kernel(x_hbm, k_hbm, v_hbm, wq_hbm, wo_hbm, w1_hbm, b1_hbm, w2_hbm, b2_hbm,
            c_hbm, wm_hbm, wm2_hbm, o_ref,
            x_v, c_v, w1_v, b1_v, w2_v, b2_v, wm_v, gb_v, wq_v, wo_v, k_v, v_v,
            q_v, p_v, o_v, t_v, th_v, w1c, b1c, scc, occ, lhs_v, sems, *, D, F, SK, W):
    col0 = SK - W
    ncb = W // 128
    NQ = HQ * DH
    nd = D // 128
    last = NPAIR - 1
    nblk = NQ // WO_G // 128
    b_late = nblk - 2 * PB
    P = functools.partial

    def wait_all(buf, sem):
        pltpu.make_async_copy(buf, buf, sems.at[sem]).wait()

    def kv_piece(is_v, pair, half, cb, sem=None):
        src, dst, s0 = (v_hbm, v_v, S_V) if is_v else (k_hbm, k_v, S_K)
        slot = pair % 2
        c = cb * 128
        if not isinstance(cb, int):
            c = pl.multiple_of(c, 128)
        return pltpu.make_async_copy(
            src.at[pair, pl.ds(half * DH, DH), pl.ds(col0 + c, 128)],
            dst.at[slot, pl.ds(half * DH, DH), pl.ds(c, 128)],
            sems.at[s0 + slot if sem is None else sem])

    def last_v_piece(half, cb):
        return kv_piece(True, last, half, cb, S_TV + _chunk_of(cb * 128, TAIL_V))

    def wm_piece(r, sec):
        idx = (slice(None), pl.ds(r, 8), pl.ds(sec * D, D))
        return pltpu.make_async_copy(wm_hbm.at[idx], wm_v.at[idx], sems.at[S_WM])

    def wq_piece(r, c):
        idx = (slice(None), pl.ds(r, 8), pl.ds(c, WQ_C))
        return pltpu.make_async_copy(wq_hbm.at[idx], wq_v.at[idx], sems.at[S_WQ])

    def wo_piece(b, r):
        part = _chunk_of(b, (b_late, PB, PB))
        idx = (pl.ds(0, WO_G - 1 if part == 1 else WO_G), b, pl.ds(r, 8), slice(None))
        return pltpu.make_async_copy(wo_hbm.at[idx], wo_v.at[idx], sems.at[S_WO + part])

    def late_wo_piece(r):
        idx = (WO_G - 1, b_late + r // 128, pl.ds(r % 128, 32), slice(None))
        return pltpu.make_async_copy(wo_hbm.at[idx], wo_v.at[idx],
                                     sems.at[S_TO + _chunk_of(r, TAIL_WO)])

    def gate_piece(r):
        return pltpu.make_async_copy(
            wm2_hbm.at[pl.ds(r, 16), pl.ds(5 * D, D)], gb_v.at[pl.ds(r, 16), :],
            sems.at[S_GB + (r >= GATE_MXU)])

    def issue(lst):
        for f, prio in lst:
            f().start(priority=prio)

    def issue_kv(is_v, pair):
        nv, npair = (False, pair + 1) if is_v else (True, pair)

        def body(cb, carry):
            kv_piece(is_v, pair, 0, cb).start(priority=0)
            kv_piece(nv, npair, 1, cb).start(priority=1)
            return carry
        lax.fori_loop(0, ncb, body, 0, unroll=4)

    wm_p = [P(wm_piece, r, s) for r in range(0, D // WM_G, 8) for s in range(5)]
    wq_p = [P(wq_piece, r, c) for r in range(0, D // WQ_G, 8) for c in range(0, NQ, WQ_C)]
    wo_p = [P(wo_piece, b, r) for b in range(nblk) for r in range(0, 128, 8)]
    seq_a = [f for l in (wm_p, wq_p, wo_p) for f in l[:len(l) // 2]]
    seq_b = [f for l in (wm_p, wq_p, wo_p) for f in l[len(l) // 2:]]
    seq_b += [P(kv_piece, False, 0, 1, cb) for cb in range(ncb)]
    head = [(f, 1) for f in seq_b[:LEAD]] + _merge(seq_a, seq_b[LEAD:])
    cut1 = LEAD + len(wm_p) + 2 * FIFO
    cut2 = cut1 + len(wq_p)

    small = [pltpu.make_async_copy(src, dst, sems.at[S_SMALL]) for src, dst in (
        (x_hbm, x_v), (c_hbm, c_v), (w1_hbm, w1_v), (b1_hbm, b1_v), (w2_hbm, w2_v),
        (b2_hbm, b2_v))]
    for cp in small:
        cp.start()
    issue(head[:cut1])
    for cp in small:
        cp.wait()
    wait_all(wm_v, S_WM)

    x = jnp.broadcast_to(x_v[...].astype(F32), (8, D))
    cc = c_v[...].astype(F32)
    sc = (cc * jax.nn.sigmoid(cc)).astype(BF16).astype(F32)
    sc8 = jnp.broadcast_to(sc, (8, D)).astype(BF16)
    mod = jnp.dot(sc8, wm_v[...].reshape(D, 5 * D), preferred_element_type=F32)
    sa, ca, ga, sb, cb_ = (mod[:, i * D:(i + 1) * D] for i in range(5))
    xm = x - _mean(x)
    h8 = (xm * lax.rsqrt(_mean(xm * xm) + EPS) * (1.0 + ca) + sa).astype(BF16)
    A = 1.0 + cb_
    Bc = sb - _mean(sb)
    A2, AB = A * A, A * Bc
    eA, eA2, eAB, eB2 = _mean(A), _mean(A2), _mean(AB), _mean(Bc * Bc)

    eye = (lax.broadcasted_iota(jnp.int32, (128, 128), 0)
           == lax.broadcasted_iota(jnp.int32, (128, 128), 1))
    ones = jnp.ones((128, 128), BF16)

    def column(rowvec):
        diag = jnp.where(eye, jnp.broadcast_to(rowvec, (128, 128)), 0.0).astype(BF16)
        return jnp.dot(diag, ones, preferred_element_type=F32)

    for r in range(GATE_MXU, D, 128):
        scc[r - GATE_MXU:r - GATE_MXU + 128, :] = column(sc[:, r:r + 128])

    w1r = w1_v[...].astype(F32)
    w2r = w2_v[...].astype(F32)
    b1r = b1_v[...].astype(F32)
    row128 = lax.broadcasted_iota(jnp.int32, (8, 128), 0)
    lin = jnp.zeros((8, 128), F32)
    for j in range(F // 128):
        sl = slice(j * 128, (j + 1) * 128)
        r1, rb, r2 = w1r[:, sl], b1r[j:j + 1, :], w2r[:, sl]
        w1c[sl, :] = column(r1) * GELU_S
        b1c[sl, :] = column(rb) * GELU_S
        t = jnp.where(row128 < 4, r1, rb) * (0.5 * r2)
        hi = t.astype(BF16).astype(F32)
        lo = (t - hi).astype(BF16).astype(F32)
        lhs_v[:, sl] = jnp.where(row128 % 4 == 0, hi, jnp.where(row128 % 4 == 1, lo, 0.0))
        lin = lin + t
    lin = jnp.sum(lin, axis=-1, keepdims=True)
    lin = lin + jnp.where(lax.broadcasted_iota(jnp.int32, (8, 1), 0) < 4, 0.0,
                          b2_v[...].astype(F32))
    lin = jnp.where(lax.broadcasted_iota(jnp.int32, (8, D), 0) % 4 == 0,
                    jnp.broadcast_to(lin, (8, D)), 0.0)

    issue(head[cut1:cut2])
    wait_all(wq_v, S_WQ)
    own = ((lax.broadcasted_iota(jnp.int32, (8, PAIR), 1) >= DH)
           == (lax.broadcasted_iota(jnp.int32, (8, PAIR), 0) % 2 == 1))
    q_all = jnp.dot(h8, wq_v[...].reshape(D, NQ), preferred_element_type=F32)
    for p in range(NPAIR):
        q_v[p] = jnp.where(own, q_all[:, p * PAIR:(p + 1) * PAIR], 0.0).astype(BF16)

    issue(head[cut2:])
    issue_kv(False, 0)
    wait_all(wo_v.at[:, pl.ds(0, b_late)], S_WO)
    wait_all(wo_v.at[pl.ds(0, WO_G - 1), pl.ds(b_late, PB)], S_WO + 1)
    wait_all(wo_v.at[:, pl.ds(b_late + PB, PB)], S_WO + 2)

    nt = (((1,), (1,)), ((), ()))

    def scores(pair):
        slot = pair % 2
        wait_all(k_v.at[slot], S_K + slot)
        s = jnp.dot(q_v[pair], k_v[slot], preferred_element_type=F32) * DH ** -0.5
        e = jnp.exp(s - jnp.max(s, axis=-1, keepdims=True))
        p_v[...] = e.astype(BF16)
        return 1.0 / jnp.sum(e, axis=-1, keepdims=True)

    def values(pair):
        slot = pair % 2
        wait_all(v_v.at[slot], S_V + slot)
        return lax.dot_general(p_v[...], v_v[slot], nt, preferred_element_type=F32)

    def project(o, inv_l, pair):
        o = jnp.where(own, o * inv_l, 0.0).astype(BF16)
        r = None
        for i in range(PB):
            j = pair * PB + i
            t = jnp.dot(o[:, i * 128:(i + 1) * 128], wo_v[j // nblk, j % nblk],
                        preferred_element_type=F32)
            r = t if r is None else r + t
        return r

    def stage(s, acc):
        issue_kv(True, s)
        inv_l = scores(s)
        issue_kv(False, s + 1)
        return acc + project(values(s), inv_l, s)

    acc = lax.fori_loop(0, last - 1, stage, jnp.zeros((8, D), F32))

    issue_kv(True, last - 1)
    inv_l = scores(last - 1)
    issue(_merge([P(kv_piece, False, last, 0, cb) for cb in range(ncb)],
                 [P(last_v_piece, 1, cb) for cb in range(ncb)]))
    o = jnp.where(own, values(last - 1) * inv_l, 0.0)
    o = o + pltpu.roll(o, 1, 0)
    for i in range(PB):
        occ[i * 128:(i + 1) * 128, :] = column(o[0:1, i * 128:(i + 1) * 128])

    va = [P(last_v_piece, 0, cb) for cb in range(ncb)]
    lw = [P(late_wo_piece, r) for r in range(0, PAIR, 32)]
    k = ncb - 2 * MOVE
    tail = _merge(va[:k] + va[k::2] + lw[0::2],
                  va[k + 1::2] + lw[1::2] + [P(gate_piece, r) for r in range(0, D, 16)])
    issue(tail[:2 * FIFO])
    inv_l = scores(last)
    xc = x + ga * (acc + pltpu.roll(acc, 1, 0))
    shift = _mean(xc)
    xc = xc - shift
    issue(tail[2 * FIFO:])

    vs = last % 2
    c0 = 0
    for ci, cw in enumerate(TAIL_V):
        wait_all(v_v.at[vs, :, pl.ds(c0, cw)], S_TV + ci)
        o = lax.dot_general(p_v[:, c0:c0 + cw], v_v[vs, :, c0:c0 + cw], nt,
                            preferred_element_type=F32)
        if ci > 0:
            o = o + o_v[...]
        if ci < len(TAIL_V) - 1:
            o_v[...] = o
        c0 += cw
    t = project(o, inv_l, last)
    xc = xc + ga * (t + pltpu.roll(t, 1, 0))

    def vpu_matvec(w, col, part=None):
        for r in range(0, w.shape[0], 16):
            prod = w[r:r + 16, :].astype(F32) * jnp.tile(col[r:r + 16, :], (1, nd))
            part = prod if part is None else part + prod
        return part

    part = None
    r0 = 0
    for ci, n in enumerate(TAIL_WO):
        rows = wo_v.at[WO_G - 1, b_late + r0 // 128, pl.ds(r0 % 128, n)]
        wait_all(rows, S_TO + ci)
        part = vpu_matvec(rows, occ.at[pl.ds(r0, n)], part)
        r0 += n
    xc = xc + ga * _sublane_allsum(part[:8] + part[8:])
    x1 = xc + shift

    xa = xc * A
    d1, e2 = _mean(xc), _mean(xc * xc)
    exa, exa2, exaa, exab = _mean(xa), _mean(xa * xa), _mean(xc * A2), _mean(xc * AB)
    r1 = lax.rsqrt(jnp.maximum(e2 - d1 * d1, 0.0) + EPS)
    mu = exa - d1 * eA
    p2 = exa2 - d1 * (2.0 * exaa - d1 * eA2) - mu * mu
    p1 = 2.0 * (exab - d1 * eAB)
    r2 = lax.rsqrt(jnp.maximum((p2 * r1 + p1) * r1 + eB2, 0.0) + EPS)
    hm = ((xa - d1 * A - mu) * r1 + Bc) * r2

    def tanh_rows(h, r, n):
        s = (jnp.tile(h, (n // 8, 1)) * jnp.tile(w1c[r:r + n, :], (1, nd))
             + jnp.tile(b1c[r:r + n, :], (1, nd)))
        return jnp.tanh(s * (s * s + GELU_K))

    def reduce_block(j, th):
        return jnp.dot(lhs_v[:, j * 128:(j + 1) * 128], th, preferred_element_type=F32)

    nb = F // 128
    R = lin
    th = None
    gate_rows = []
    for j in range(nb):
        if j == GATE_AT:
            wait_all(gb_v.at[pl.ds(0, GATE_MXU)], S_GB)
            R = R + reduce_block(j - 1, th_v[...])
            gate_rows = list(range(0, GATE_MXU, 128))
        if j + 1 in (GATE_AT, nb):
            z = th[0:8, 0:128]
            for i in range(1, nd):
                z = z + th[0:8, i * 128:(i + 1) * 128]
            hd = hm + jnp.tile(0.0 * z, (1, nd))
            for r in range(0, 128, 8):
                th_v[r:r + 8, :] = tanh_rows(hd, j * 128 + r, 8)
        else:
            th = tanh_rows(hm, j * 128, 128)
            R = R + reduce_block(j, th)
            for r in gate_rows[:2]:
                t_v[r // 128] = jnp.dot(sc8[:, r:r + 128], gb_v[r:r + 128, :],
                                        preferred_element_type=F32)
            gate_rows = gate_rows[2:]
    assert not gate_rows
    rows = gb_v.at[pl.ds(GATE_MXU, D - GATE_MXU)]
    wait_all(rows, S_GB + 1)
    R = R + reduce_block(nb - 1, th_v[...])
    part = vpu_matvec(rows, scc)
    gb = _sublane_allsum(part[:8] + part[8:])
    for i in range(GATE_MXU // 128):
        gb = gb + t_v[i]
    R = R + pltpu.roll(R, 7, 0)
    y = hm * R + pltpu.roll(R, 4, 0)
    o_ref[...] = (x1 + gb * y)[0:1].astype(o_ref.dtype)


@jax.jit
def pallas_adaLN_cond__sliding_block_cached__mixer_token_mlp__decode_kernel(
    A_x: jax.Array,
    A_k_cache: jax.Array,
    A_v_cache: jax.Array,
    A_wq: jax.Array,
    A_wo: jax.Array,
    B_x: jax.Array,
    B_w1: jax.Array,
    B_b1: jax.Array,
    B_w2: jax.Array,
    B_b2: jax.Array,
    c: jax.Array,
    w_mod: jax.Array,
):
    B, SQ, D = A_x.shape
    _, HKV, SK, dh = A_k_cache.shape
    S, F = B_w1.shape
    assert B == 1 and SQ == 1 and S == 1 and HKV == HQ and dh == DH
    W = min(4096, max(256, SK // 4))
    assert sum(TAIL_V) == W and sum(TAIL_WO) == PAIR
    NQ = HQ * DH

    kt = jnp.swapaxes(A_k_cache, 2, 3).reshape(NPAIR, PAIR, SK)
    vt = jnp.swapaxes(A_v_cache, 2, 3).reshape(NPAIR, PAIR, SK)
    args = (
        A_x.reshape(1, D), kt, vt, A_wq.reshape(WQ_G, D // WQ_G, NQ),
        A_wo.reshape(WO_G, NQ // WO_G // 128, 128, D),
        B_w1, B_b1.reshape(F // 128, 128), B_w2.reshape(1, F), B_b2.reshape(1, 1),
        c, w_mod.reshape(WM_G, D // WM_G, 6 * D), w_mod,
    )
    out = pl.pallas_call(
        functools.partial(_kernel, D=D, F=F, SK=SK, W=W),
        out_shape=jax.ShapeDtypeStruct((1, D), A_x.dtype),
        in_specs=[pl.BlockSpec(memory_space=pl.ANY)] * len(args),
        out_specs=pl.BlockSpec(memory_space=pltpu.VMEM),
        scratch_shapes=[
            pltpu.VMEM((1, D), BF16),
            pltpu.VMEM((1, D), BF16),
            pltpu.VMEM((1, F), BF16),
            pltpu.VMEM((F // 128, 128), BF16),
            pltpu.VMEM((1, F), BF16),
            pltpu.VMEM((1, 1), BF16),
            pltpu.VMEM((WM_G, D // WM_G, 5 * D), BF16),
            pltpu.VMEM((D, D), BF16),
            pltpu.VMEM((WQ_G, D // WQ_G, NQ), BF16),
            pltpu.VMEM((WO_G, NQ // WO_G // 128, 128, D), BF16),
            pltpu.VMEM((2, PAIR, W), BF16),
            pltpu.VMEM((2, PAIR, W), BF16),
            pltpu.VMEM((NPAIR, 8, PAIR), BF16),
            pltpu.VMEM((8, W), BF16),
            pltpu.VMEM((8, PAIR), F32),
            pltpu.VMEM((GATE_MXU // 128, 8, D), F32),
            pltpu.VMEM((128, D), F32),
            pltpu.VMEM((F, 128), F32),
            pltpu.VMEM((F, 128), F32),
            pltpu.VMEM((D - GATE_MXU, 128), F32),
            pltpu.VMEM((PAIR, 128), F32),
            pltpu.VMEM((8, F), F32),
            pltpu.SemaphoreType.DMA((N_SEMS,)),
        ],
        compiler_params=pltpu.CompilerParams(
            vmem_limit_bytes=64 * 1024 * 1024,
            disable_bounds_checks=True,
            disable_semaphore_checks=True,
        ),
    )(*args)
    return out.reshape(B, SQ, D)
```

```python
import functools
import math

import jax
import jax.numpy as jnp
from jax import lax
import jax.experimental.pallas as pl
import jax.experimental.pallas.tpu as pltpu

F32 = jnp.float32
BF16 = jnp.bfloat16

HQ = 32
DH = 192
PAIR = 2 * DH
NPAIR = HQ // 2
PB = PAIR // 128
EPS = 1e-5
GELU_C = math.sqrt(2.0 / math.pi)
GELU_A = 0.044715
GELU_S = (GELU_C * GELU_A) ** (1.0 / 3.0)
GELU_K = GELU_C / GELU_S

LEAD = 32
FIFO = 28
WM_G = 4
WQ_G, WQ_C = 5, 512
WO_G = 3
MOVE = 3
TAIL_V = (2048, 1024, 512, 512)
TAIL_WO = (128, 128, 64, 64)
TAIL_GATE = (192, 192, 192, 64)
BLK = 96
AT = 2
FIRST, LOOK = 2, 3
SPLIT = 24

S_SMALL, S_WM, S_WQ = 0, 1, 2
S_WO = 3
S_K, S_V = 6, 8
S_TV = 10
S_TO = S_TV + len(TAIL_V)
S_GB = S_TO + len(TAIL_WO)
N_SEMS = S_GB + len(TAIL_GATE)


def _mean(t):
    return jnp.mean(t, axis=-1, keepdims=True)


def _chunk_of(pos, chunks):
    end = 0
    for ci, n in enumerate(chunks):
        end += n
        if pos < end:
            return ci
    raise ValueError(pos)


def _sublane_allsum(t):
    t = t + pltpu.roll(t, 4, 0)
    t = t + pltpu.roll(t, 2, 0)
    return t + pltpu.roll(t, 1, 0)


def _split3(t):
    hi = t.astype(BF16).astype(F32)
    r = t - hi
    mid = r.astype(BF16).astype(F32)
    return hi, mid, (r - mid).astype(BF16).astype(F32)


def _rows(row, vals):
    out = jnp.zeros(row.shape, F32)
    done = []
    for v in vals:
        if any(v is d for d in done):
            continue
        done.append(v)
        m = None
        for i, u in enumerate(vals):
            if u is v:
                m = (row == i) if m is None else m | (row == i)
        out = jnp.where(m, v, out)
    return out


def _merge(a, b):
    out = []
    for i in range(max(len(a), len(b))):
        if i < len(a):
            out.append((a[i], 0))
        if i < len(b):
            out.append((b[i], 1))
    return out


def _kernel(x_hbm, k_hbm, v_hbm, wq_hbm, wo_hbm, w1_hbm, b1_hbm, w2_hbm, b2_hbm,
            c_hbm, wm_hbm, wm2_hbm, o_ref,
            x_v, c_v, w1_v, b1_v, w2_v, b2_v, wm_v, gb_v, wq_v, wo_v, k_v, v_v,
            q_v, p_v, o_v, w1c, b1c, cz_v, scc, occ, lhs_v, sems, *, D, F, SK, W):
    col0 = SK - W
    ncb = W // 128
    NQ = HQ * DH
    nd = D // 128
    last = NPAIR - 1
    nblk = NQ // WO_G // 128
    b_late = nblk - 2 * PB
    P = functools.partial

    def wait_all(buf, sem):
        pltpu.make_async_copy(buf, buf, sems.at[sem]).wait()

    def kv_piece(is_v, pair, half, cb, sem=None):
        src, dst, s0 = (v_hbm, v_v, S_V) if is_v else (k_hbm, k_v, S_K)
        slot = pair % 2
        c = cb * 128
        if not isinstance(cb, int):
            c = pl.multiple_of(c, 128)
        return pltpu.make_async_copy(
            src.at[pair, pl.ds(half * DH, DH), pl.ds(col0 + c, 128)],
            dst.at[slot, pl.ds(half * DH, DH), pl.ds(c, 128)],
            sems.at[s0 + slot if sem is None else sem])

    def last_v_piece(half, cb):
        return kv_piece(True, last, half, cb, S_TV + _chunk_of(cb * 128, TAIL_V))

    def wm_piece(r, sec):
        idx = (slice(None), pl.ds(r, 8), pl.ds(sec * D, D))
        return pltpu.make_async_copy(wm_hbm.at[idx], wm_v.at[idx], sems.at[S_WM])

    def wq_piece(r, c):
        idx = (slice(None), pl.ds(r, 8), pl.ds(c, WQ_C))
        return pltpu.make_async_copy(wq_hbm.at[idx], wq_v.at[idx], sems.at[S_WQ])

    def wo_piece(b, r):
        part = _chunk_of(b, (b_late, PB, PB))
        idx = (pl.ds(0, WO_G - 1 if part == 1 else WO_G), b, pl.ds(r, 8), slice(None))
        return pltpu.make_async_copy(wo_hbm.at[idx], wo_v.at[idx], sems.at[S_WO + part])

    def late_wo_piece(r):
        idx = (WO_G - 1, b_late + r // 128, pl.ds(r % 128, 32), slice(None))
        return pltpu.make_async_copy(wo_hbm.at[idx], wo_v.at[idx],
                                     sems.at[S_TO + _chunk_of(r, TAIL_WO)])

    def gate_piece(r):
        return pltpu.make_async_copy(
            wm2_hbm.at[pl.ds(r, 16), pl.ds(5 * D, D)], gb_v.at[pl.ds(r, 16), :],
            sems.at[S_GB + _chunk_of(r, TAIL_GATE)])

    def issue(lst):
        for f, prio in lst:
            f().start(priority=prio)

    def issue_kv(is_v, pair):
        nv, npair = (False, pair + 1) if is_v else (True, pair)

        def body(cb, carry):
            kv_piece(is_v, pair, 0, cb).start(priority=0)
            kv_piece(nv, npair, 1, cb).start(priority=1)
            return carry
        lax.fori_loop(0, ncb, body, 0, unroll=4)

    wm_p = [P(wm_piece, r, s) for r in range(0, D // WM_G, 8) for s in range(5)]
    wq_p = [P(wq_piece, r, c) for r in range(0, D // WQ_G, 8) for c in range(0, NQ, WQ_C)]
    wo_p = [P(wo_piece, b, r) for b in range(nblk) for r in range(0, 128, 8)]
    seq_a = [f for l in (wm_p, wq_p, wo_p) for f in l[:len(l) // 2]]
    seq_b = [f for l in (wm_p, wq_p, wo_p) for f in l[len(l) // 2:]]
    seq_b += [P(kv_piece, False, 0, 1, cb) for cb in range(ncb)]
    head = [(f, 1) for f in seq_b[:LEAD]] + _merge(seq_a, seq_b[LEAD:])
    cut1 = LEAD + len(wm_p) + 2 * FIFO
    cut2 = cut1 + len(wq_p)

    small = [pltpu.make_async_copy(src, dst, sems.at[S_SMALL]) for src, dst in (
        (x_hbm, x_v), (c_hbm, c_v), (w1_hbm, w1_v), (b1_hbm, b1_v), (w2_hbm, w2_v),
        (b2_hbm, b2_v))]
    for cp in small:
        cp.start()
    issue(head[:cut1])
    for cp in small:
        cp.wait()
    wait_all(wm_v, S_WM)

    x = jnp.broadcast_to(x_v[...].astype(F32), (8, D))
    cc = c_v[...].astype(F32)
    sc = (cc * jax.nn.sigmoid(cc)).astype(BF16).astype(F32)
    sc8 = jnp.broadcast_to(sc, (8, D)).astype(BF16)
    mod = jnp.dot(sc8, wm_v[...].reshape(D, 5 * D), preferred_element_type=F32)
    sa, ca, ga, sb, cb_ = (mod[:, i * D:(i + 1) * D] for i in range(5))
    xm = x - _mean(x)
    h8 = (xm * lax.rsqrt(_mean(xm * xm) + EPS) * (1.0 + ca) + sa).astype(BF16)
    A = 1.0 + cb_
    Bc = sb - _mean(sb)
    A2, AB = A * A, A * Bc
    eA, eA2, eAB, eB2 = _mean(A), _mean(A2), _mean(AB), _mean(Bc * Bc)

    eye = (lax.broadcasted_iota(jnp.int32, (128, 128), 0)
           == lax.broadcasted_iota(jnp.int32, (128, 128), 1))
    ones = jnp.ones((128, 128), BF16)
    ident = jnp.where(eye, 1.0, 0.0)
    nt = (((1,), (1,)), ((), ()))

    def column(rowvec):
        diag = jnp.where(eye, jnp.broadcast_to(rowvec, (128, 128)), 0.0).astype(BF16)
        return jnp.dot(diag, ones, preferred_element_type=F32)

    for r in range(0, D, 128):
        scc[r:r + 128, :] = column(sc[:, r:r + 128])

    w1r = w1_v[...].astype(F32)
    w2r = w2_v[...].astype(F32)
    b1r = b1_v[...].astype(F32)
    row128 = lax.broadcasted_iota(jnp.int32, (8, 128), 0)
    lin = jnp.zeros((8, 128), F32)
    for j in range(F // 128):
        sl = slice(j * 128, (j + 1) * 128)
        r1, rb, r2 = w1r[:, sl], b1r[j:j + 1, :], w2r[:, sl]
        w1c[sl, :] = column(r1) * GELU_S
        b1c[sl, :] = column(rb) * GELU_S
        t = jnp.where(row128 < 4, r1, rb) * (0.5 * r2)
        hi = t.astype(BF16).astype(F32)
        lo = (t - hi).astype(BF16).astype(F32)
        lhs_v[:, sl] = jnp.where(row128 % 4 == 0, hi, jnp.where(row128 % 4 == 1, lo, 0.0))
        lin = lin + t
        w, b = r1 * GELU_S, rb * GELU_S
        c0 = _split3(b * (b * b + GELU_K))
        groups = []
        for i, cf in enumerate((w * (3.0 * b * b + GELU_K), 3.0 * w * w * b, w * w * w)):
            ch, cm, cl = _split3(cf)
            groups.append(_rows(row128, (ch, ch, cm, ch, cl, cm, c0[i])))
        cz_v[sl, :] = lax.dot_general(ident, jnp.concatenate(groups, axis=0), nt,
                                      preferred_element_type=F32)
    lin = jnp.sum(lin, axis=-1, keepdims=True)
    lin = lin + jnp.where(lax.broadcasted_iota(jnp.int32, (8, 1), 0) < 4, 0.0,
                          b2_v[...].astype(F32))
    lin = jnp.where(lax.broadcasted_iota(jnp.int32, (8, D), 0) % 4 == 0,
                    jnp.broadcast_to(lin, (8, D)), 0.0)

    issue(head[cut1:cut2])
    wait_all(wq_v, S_WQ)
    own = ((lax.broadcasted_iota(jnp.int32, (8, PAIR), 1) >= DH)
           == (lax.broadcasted_iota(jnp.int32, (8, PAIR), 0) % 2 == 1))
    q_all = jnp.dot(h8, wq_v[...].reshape(D, NQ), preferred_element_type=F32)
    for p in range(NPAIR):
        q_v[p] = jnp.where(own, q_all[:, p * PAIR:(p + 1) * PAIR], 0.0).astype(BF16)

    issue(head[cut2:])
    issue_kv(False, 0)
    wait_all(wo_v.at[:, pl.ds(0, b_late)], S_WO)
    wait_all(wo_v.at[pl.ds(0, WO_G - 1), pl.ds(b_late, PB)], S_WO + 1)
    wait_all(wo_v.at[:, pl.ds(b_late + PB, PB)], S_WO + 2)

    def scores(pair):
        slot = pair % 2
        wait_all(k_v.at[slot], S_K + slot)
        s = jnp.dot(q_v[pair], k_v[slot], preferred_element_type=F32) * DH ** -0.5
        e = jnp.exp(s - jnp.max(s, axis=-1, keepdims=True))
        p_v[...] = e.astype(BF16)
        return 1.0 / jnp.sum(e, axis=-1, keepdims=True)

    def values(pair):
        slot = pair % 2
        wait_all(v_v.at[slot], S_V + slot)
        return lax.dot_general(p_v[...], v_v[slot], nt, preferred_element_type=F32)

    def project(o, inv_l, pair):
        o = jnp.where(own, o * inv_l, 0.0).astype(BF16)
        r = None
        for i in range(PB):
            j = pair * PB + i
            t = jnp.dot(o[:, i * 128:(i + 1) * 128], wo_v[j // nblk, j % nblk],
                        preferred_element_type=F32)
            r = t if r is None else r + t
        return r

    def stage(s, acc):
        issue_kv(True, s)
        inv_l = scores(s)
        issue_kv(False, s + 1)
        return acc + project(values(s), inv_l, s)

    acc = lax.fori_loop(0, last - 1, stage, jnp.zeros((8, D), F32))

    issue_kv(True, last - 1)
    inv_l = scores(last - 1)
    issue(_merge([P(kv_piece, False, last, 0, cb) for cb in range(ncb)],
                 [P(last_v_piece, 1, cb) for cb in range(ncb)]))
    o = jnp.where(own, values(last - 1) * inv_l, 0.0)
    o = o + pltpu.roll(o, 1, 0)
    for i in range(PB):
        occ[i * 128:(i + 1) * 128, :] = column(o[0:1, i * 128:(i + 1) * 128])

    va = [P(last_v_piece, 0, cb) for cb in range(ncb)]
    lw = [P(late_wo_piece, r) for r in range(0, PAIR, 32)]
    k = ncb - 2 * MOVE
    tail = _merge(va[:k] + va[k::2] + lw[0::2],
                  va[k + 1::2] + lw[1::2] + [P(gate_piece, r) for r in range(0, D, 16)])
    issue(tail[:2 * FIFO])
    inv_l = scores(last)
    xc = x + ga * (acc + pltpu.roll(acc, 1, 0))
    shift = _mean(xc)
    xc = xc - shift

    vs = last % 2
    c0 = 0
    for ci, cw in enumerate(TAIL_V):
        wait_all(v_v.at[vs, :, pl.ds(c0, cw)], S_TV + ci)
        if ci == 0:
            issue(tail[2 * FIFO:])
        o = lax.dot_general(p_v[:, c0:c0 + cw], v_v[vs, :, c0:c0 + cw], nt,
                            preferred_element_type=F32)
        if ci > 0:
            o = o + o_v[...]
        if ci < len(TAIL_V) - 1:
            o_v[...] = o
        c0 += cw
    t = project(o, inv_l, last)
    xc = xc + ga * (t + pltpu.roll(t, 1, 0))

    def vpu_matvec(w, col, part=None):
        for r in range(0, w.shape[0], 16):
            prod = w[r:r + 16, :].astype(F32) * jnp.tile(col[r:r + 16, :], (1, nd))
            part = prod if part is None else part + prod
        return part

    part = None
    r0 = 0
    for ci, n in enumerate(TAIL_WO):
        rows = wo_v.at[WO_G - 1, b_late + r0 // 128, pl.ds(r0 % 128, n)]
        wait_all(rows, S_TO + ci)
        part = vpu_matvec(rows, occ.at[pl.ds(r0, n)], part)
        r0 += n
    xc = xc + ga * _sublane_allsum(part[:8] + part[8:])
    x1 = xc + shift

    xa = xc * A
    d1, e2 = _mean(xc), _mean(xc * xc)
    exa, exa2, exaa, exab = _mean(xa), _mean(xa * xa), _mean(xc * A2), _mean(xc * AB)
    r1 = lax.rsqrt(jnp.maximum(e2 - d1 * d1, 0.0) + EPS)
    mu = exa - d1 * eA
    p2 = exa2 - d1 * (2.0 * exaa - d1 * eA2) - mu * mu
    p1 = 2.0 * (exab - d1 * eAB)
    r2 = lax.rsqrt(jnp.maximum((p2 * r1 + p1) * r1 + eB2, 0.0) + EPS)
    hm = ((xa - d1 * A - mu) * r1 + Bc) * r2

    rowp = lax.broadcasted_iota(jnp.int32, (8, AT * 128), 0)
    h1 = hm[:, :AT * 128]
    h2 = h1 * h1
    groups = []
    for pw in (h1, h2, h2 * h1):
        ph, pm, pl_ = _split3(pw)
        groups.append(_rows(rowp, (ph, pm, ph, pl_, ph, pm, 1.0)))
    hp = jnp.concatenate(groups, axis=0)

    def mxu_arg(j):
        return jnp.concatenate([jnp.concatenate([
            jnp.dot(cz_v[r:r + SPLIT, :], hp[:, t * 128:(t + 1) * 128], preferred_element_type=F32)
            for r in range(j * BLK, (j + 1) * BLK, SPLIT)], axis=0) for t in range(AT)], axis=1)

    nb = F // BLK
    R = lin
    ahead = {}
    for j in range(FIRST, LOOK):
        ahead[j] = mxu_arg(j)
    for j in range(nb):
        if j + LOOK < nb:
            ahead[j + LOOK] = mxu_arg(j + LOOK)
        sl = slice(j * BLK, (j + 1) * BLK)
        k = AT if j in ahead else 0
        s = (jnp.tile(hm[:, k * 128:], (BLK // 8, 1)) * jnp.tile(w1c[sl, :], (1, nd - k))
             + jnp.tile(b1c[sl, :], (1, nd - k)))
        z = s * (s * s + GELU_K)
        if k:
            z = jnp.concatenate([ahead.pop(j), z], axis=1)
        R = R + jnp.dot(lhs_v[:, sl], jnp.tanh(z), preferred_element_type=F32)
    R = R + pltpu.roll(R, 7, 0)
    y = hm * R + pltpu.roll(R, 4, 0)

    part = None
    r0 = 0
    for ci, n in enumerate(TAIL_GATE):
        rows = gb_v.at[pl.ds(r0, n)]
        wait_all(rows, S_GB + ci)
        part = vpu_matvec(rows, scc.at[pl.ds(r0, n)], part)
        r0 += n
    gb = _sublane_allsum(part[:8] + part[8:])
    o_ref[...] = (x1 + gb * y)[0:1].astype(o_ref.dtype)


@jax.jit
def pallas_adaLN_cond__sliding_block_cached__mixer_token_mlp__decode_kernel(
    A_x: jax.Array,
    A_k_cache: jax.Array,
    A_v_cache: jax.Array,
    A_wq: jax.Array,
    A_wo: jax.Array,
    B_x: jax.Array,
    B_w1: jax.Array,
    B_b1: jax.Array,
    B_w2: jax.Array,
    B_b2: jax.Array,
    c: jax.Array,
    w_mod: jax.Array,
):
    B, SQ, D = A_x.shape
    _, HKV, SK, dh = A_k_cache.shape
    S, F = B_w1.shape
    assert B == 1 and SQ == 1 and S == 1 and HKV == HQ and dh == DH
    W = min(4096, max(256, SK // 4))
    assert sum(TAIL_V) == W and sum(TAIL_WO) == PAIR and sum(TAIL_GATE) == D
    NQ = HQ * DH

    kt = jnp.swapaxes(A_k_cache, 2, 3).reshape(NPAIR, PAIR, SK)
    vt = jnp.swapaxes(A_v_cache, 2, 3).reshape(NPAIR, PAIR, SK)
    args = (
        A_x.reshape(1, D), kt, vt, A_wq.reshape(WQ_G, D // WQ_G, NQ),
        A_wo.reshape(WO_G, NQ // WO_G // 128, 128, D),
        B_w1, B_b1.reshape(F // 128, 128), B_w2.reshape(1, F), B_b2.reshape(1, 1),
        c, w_mod.reshape(WM_G, D // WM_G, 6 * D), w_mod,
    )
    out = pl.pallas_call(
        functools.partial(_kernel, D=D, F=F, SK=SK, W=W),
        out_shape=jax.ShapeDtypeStruct((1, D), A_x.dtype),
        in_specs=[pl.BlockSpec(memory_space=pl.ANY)] * len(args),
        out_specs=pl.BlockSpec(memory_space=pltpu.VMEM),
        scratch_shapes=[
            pltpu.VMEM((1, D), BF16),
            pltpu.VMEM((1, D), BF16),
            pltpu.VMEM((1, F), BF16),
            pltpu.VMEM((F // 128, 128), BF16),
            pltpu.VMEM((1, F), BF16),
            pltpu.VMEM((1, 1), BF16),
            pltpu.VMEM((WM_G, D // WM_G, 5 * D), BF16),
            pltpu.VMEM((D, D), BF16),
            pltpu.VMEM((WQ_G, D // WQ_G, NQ), BF16),
            pltpu.VMEM((WO_G, NQ // WO_G // 128, 128, D), BF16),
            pltpu.VMEM((2, PAIR, W), BF16),
            pltpu.VMEM((2, PAIR, W), BF16),
            pltpu.VMEM((NPAIR, 8, PAIR), BF16),
            pltpu.VMEM((8, W), BF16),
            pltpu.VMEM((8, PAIR), F32),
            pltpu.VMEM((F, 128), F32),
            pltpu.VMEM((F, 128), F32),
            pltpu.VMEM((F, 24), F32),
            pltpu.VMEM((D, 128), F32),
            pltpu.VMEM((PAIR, 128), F32),
            pltpu.VMEM((8, F), F32),
            pltpu.SemaphoreType.DMA((N_SEMS,)),
        ],
        compiler_params=pltpu.CompilerParams(
            vmem_limit_bytes=64 * 1024 * 1024,
            disable_bounds_checks=True,
            disable_semaphore_checks=True,
        ),
    )(*args)
    return out.reshape(B, SQ, D)
```

```python
import functools
import math

import jax
import jax.numpy as jnp
from jax import lax
import jax.experimental.pallas as pl
import jax.experimental.pallas.tpu as pltpu

F32 = jnp.float32
BF16 = jnp.bfloat16

HQ = 32
DH = 192
PAIR = 2 * DH
NPAIR = HQ // 2
PB = PAIR // 128
EPS = 1e-5
GELU_C = math.sqrt(2.0 / math.pi)
GELU_A = 0.044715
GELU_S = (GELU_C * GELU_A) ** (1.0 / 3.0)
GELU_K = GELU_C / GELU_S

LEAD = 32
FIFO = 28
WM_G = 4
WQ_G, WQ_C = 5, 512
WO_G = 3
MOVE = 3
TAIL_V = (2048, 1024, 512, 512)
TAIL_WO = (128, 128, 64, 64)
TAIL_GATE = (448, 96, 64, 32)
BLK = 96
AT = 2
FIRST, LOOK = 2, 3
SPLIT = 24
CARRY = 2

S_SMALL, S_WM, S_WQ = 0, 1, 2
S_WO = 3
S_K, S_V = 6, 8
S_TV = 10
S_TO = S_TV + len(TAIL_V)
S_GB = S_TO + len(TAIL_WO)
N_SEMS = S_GB + len(TAIL_GATE)


def _mean(t):
    return jnp.mean(t, axis=-1, keepdims=True)


def _chunk_of(pos, chunks):
    end = 0
    for ci, n in enumerate(chunks):
        end += n
        if pos < end:
            return ci
    raise ValueError(pos)


def _sublane_allsum(t):
    t = t + pltpu.roll(t, 4, 0)
    t = t + pltpu.roll(t, 2, 0)
    return t + pltpu.roll(t, 1, 0)


def _split3(t):
    hi = t.astype(BF16).astype(F32)
    r = t - hi
    mid = r.astype(BF16).astype(F32)
    return hi, mid, (r - mid).astype(BF16).astype(F32)


def _rows(row, vals):
    out = jnp.zeros(row.shape, F32)
    done = []
    for v in vals:
        if any(v is d for d in done):
            continue
        done.append(v)
        m = None
        for i, u in enumerate(vals):
            if u is v:
                m = (row == i) if m is None else m | (row == i)
        out = jnp.where(m, v, out)
    return out


def _merge(a, b):
    out = []
    for i in range(max(len(a), len(b))):
        if i < len(a):
            out.append((a[i], 0))
        if i < len(b):
            out.append((b[i], 1))
    return out


def _kernel(x_hbm, k_hbm, v_hbm, wq_hbm, wo_hbm, w1_hbm, b1_hbm, w2_hbm, b2_hbm,
            c_hbm, wm_hbm, wm2_hbm, o_ref,
            x_v, c_v, w1_v, b1_v, w2_v, b2_v, wm_v, gb_v, wq_v, wo_v, k_v, v_v,
            q_v, p_v, o_v, th_v, w1c, b1c, cz_v, scc, occ, lhs_v, sems, *, D, F, SK, W):
    col0 = SK - W
    ncb = W // 128
    NQ = HQ * DH
    nd = D // 128
    last = NPAIR - 1
    nblk = NQ // WO_G // 128
    b_late = nblk - 2 * PB
    P = functools.partial

    def wait_all(buf, sem):
        pltpu.make_async_copy(buf, buf, sems.at[sem]).wait()

    def kv_piece(is_v, pair, half, cb, sem=None):
        src, dst, s0 = (v_hbm, v_v, S_V) if is_v else (k_hbm, k_v, S_K)
        slot = pair % 2
        c = cb * 128
        if not isinstance(cb, int):
            c = pl.multiple_of(c, 128)
        return pltpu.make_async_copy(
            src.at[pair, pl.ds(half * DH, DH), pl.ds(col0 + c, 128)],
            dst.at[slot, pl.ds(half * DH, DH), pl.ds(c, 128)],
            sems.at[s0 + slot if sem is None else sem])

    def last_v_piece(half, cb):
        return kv_piece(True, last, half, cb, S_TV + _chunk_of(cb * 128, TAIL_V))

    def wm_piece(r, sec):
        idx = (slice(None), pl.ds(r, 8), pl.ds(sec * D, D))
        return pltpu.make_async_copy(wm_hbm.at[idx], wm_v.at[idx], sems.at[S_WM])

    def wq_piece(r, c):
        idx = (slice(None), pl.ds(r, 8), pl.ds(c, WQ_C))
        return pltpu.make_async_copy(wq_hbm.at[idx], wq_v.at[idx], sems.at[S_WQ])

    def wo_piece(b, r):
        part = _chunk_of(b, (b_late, PB, PB))
        idx = (pl.ds(0, WO_G - 1 if part == 1 else WO_G), b, pl.ds(r, 8), slice(None))
        return pltpu.make_async_copy(wo_hbm.at[idx], wo_v.at[idx], sems.at[S_WO + part])

    def late_wo_piece(r):
        idx = (WO_G - 1, b_late + r // 128, pl.ds(r % 128, 32), slice(None))
        return pltpu.make_async_copy(wo_hbm.at[idx], wo_v.at[idx],
                                     sems.at[S_TO + _chunk_of(r, TAIL_WO)])

    def gate_piece(r):
        return pltpu.make_async_copy(
            wm2_hbm.at[pl.ds(r, 16), pl.ds(5 * D, D)], gb_v.at[pl.ds(r, 16), :],
            sems.at[S_GB + _chunk_of(r, TAIL_GATE)])

    def issue(lst):
        for f, prio in lst:
            f().start(priority=prio)

    def issue_kv(is_v, pair):
        nv, npair = (False, pair + 1) if is_v else (True, pair)

        def body(cb, carry):
            kv_piece(is_v, pair, 0, cb).start(priority=0)
            kv_piece(nv, npair, 1, cb).start(priority=1)
            return carry
        lax.fori_loop(0, ncb, body, 0, unroll=4)

    wm_p = [P(wm_piece, r, s) for r in range(0, D // WM_G, 8) for s in range(5)]
    wq_p = [P(wq_piece, r, c) for r in range(0, D // WQ_G, 8) for c in range(0, NQ, WQ_C)]
    wo_p = [P(wo_piece, b, r) for b in range(nblk) for r in range(0, 128, 8)]
    seq_a = [f for l in (wm_p, wq_p, wo_p) for f in l[:len(l) // 2]]
    seq_b = [f for l in (wm_p, wq_p, wo_p) for f in l[len(l) // 2:]]
    seq_b += [P(kv_piece, False, 0, 1, cb) for cb in range(ncb)]
    head = [(f, 1) for f in seq_b[:LEAD]] + _merge(seq_a, seq_b[LEAD:])
    cut1 = LEAD + len(wm_p) + 2 * FIFO
    cut2 = cut1 + len(wq_p)

    small = [pltpu.make_async_copy(src, dst, sems.at[S_SMALL]) for src, dst in (
        (x_hbm, x_v), (c_hbm, c_v), (w1_hbm, w1_v), (b1_hbm, b1_v), (w2_hbm, w2_v),
        (b2_hbm, b2_v))]
    for cp in small:
        cp.start()
    issue(head[:cut1])
    for cp in small:
        cp.wait()
    wait_all(wm_v, S_WM)

    x = jnp.broadcast_to(x_v[...].astype(F32), (8, D))
    cc = c_v[...].astype(F32)
    sc = (cc * jax.nn.sigmoid(cc)).astype(BF16).astype(F32)
    sc8 = jnp.broadcast_to(sc, (8, D)).astype(BF16)
    mod = jnp.dot(sc8, wm_v[...].reshape(D, 5 * D), preferred_element_type=F32)
    sa, ca, ga, sb, cb_ = (mod[:, i * D:(i + 1) * D] for i in range(5))
    xm = x - _mean(x)
    h8 = (xm * lax.rsqrt(_mean(xm * xm) + EPS) * (1.0 + ca) + sa).astype(BF16)
    A = 1.0 + cb_
    Bc = sb - _mean(sb)
    A2, AB = A * A, A * Bc
    eA, eA2, eAB, eB2 = _mean(A), _mean(A2), _mean(AB), _mean(Bc * Bc)

    eye = (lax.broadcasted_iota(jnp.int32, (128, 128), 0)
           == lax.broadcasted_iota(jnp.int32, (128, 128), 1))
    ones = jnp.ones((128, 128), BF16)
    ident = jnp.where(eye, 1.0, 0.0)
    nt = (((1,), (1,)), ((), ()))

    def column(rowvec):
        diag = jnp.where(eye, jnp.broadcast_to(rowvec, (128, 128)), 0.0).astype(BF16)
        return jnp.dot(diag, ones, preferred_element_type=F32)

    for r in range(0, D, 128):
        scc[r:r + 128, :] = column(sc[:, r:r + 128])

    w1r = w1_v[...].astype(F32)
    w2r = w2_v[...].astype(F32)
    b1r = b1_v[...].astype(F32)
    row128 = lax.broadcasted_iota(jnp.int32, (8, 128), 0)
    lin = jnp.zeros((8, 128), F32)
    lhs = []
    for j in range(F // 128):
        sl = slice(j * 128, (j + 1) * 128)
        r1, rb, r2 = w1r[:, sl], b1r[j:j + 1, :], w2r[:, sl]
        w1c[sl, :] = column(r1) * GELU_S
        b1c[sl, :] = column(rb) * GELU_S
        t = jnp.where(row128 < 4, r1, rb) * (0.5 * r2)
        hi = t.astype(BF16).astype(F32)
        lo = (t - hi).astype(BF16).astype(F32)
        lhs.append(jnp.where(row128 % 4 == 0, hi, jnp.where(row128 % 4 == 1, lo, 0.0)))
        lin = lin + t
        w, b = r1 * GELU_S, rb * GELU_S
        c0 = _split3(b * (b * b + GELU_K))
        groups = []
        for i, cf in enumerate((w * (3.0 * b * b + GELU_K), 3.0 * w * w * b, w * w * w)):
            ch, cm, cl = _split3(cf)
            groups.append(_rows(row128, (ch, ch, cm, ch, cl, cm, c0[i])))
        cz_v[sl, :] = lax.dot_general(ident, jnp.concatenate(groups, axis=0), nt,
                                      preferred_element_type=F32)
    lhs = jnp.concatenate(lhs, axis=1)
    for j in range(F // BLK):
        lhs_v[j] = lhs[:, j * BLK:(j + 1) * BLK]
    lin = jnp.sum(lin, axis=-1, keepdims=True)
    lin = lin + jnp.where(lax.broadcasted_iota(jnp.int32, (8, 1), 0) < 4, 0.0,
                          b2_v[...].astype(F32))
    lin = jnp.where(lax.broadcasted_iota(jnp.int32, (8, D), 0) % 4 == 0,
                    jnp.broadcast_to(lin, (8, D)), 0.0)

    issue(head[cut1:cut2])
    wait_all(wq_v, S_WQ)
    own = ((lax.broadcasted_iota(jnp.int32, (8, PAIR), 1) >= DH)
           == (lax.broadcasted_iota(jnp.int32, (8, PAIR), 0) % 2 == 1))
    q_all = jnp.dot(h8, wq_v[...].reshape(D, NQ), preferred_element_type=F32)
    for p in range(NPAIR):
        q_v[p] = jnp.where(own, q_all[:, p * PAIR:(p + 1) * PAIR], 0.0).astype(BF16)

    issue(head[cut2:])
    issue_kv(False, 0)
    wait_all(wo_v.at[:, pl.ds(0, b_late)], S_WO)
    wait_all(wo_v.at[pl.ds(0, WO_G - 1), pl.ds(b_late, PB)], S_WO + 1)
    wait_all(wo_v.at[:, pl.ds(b_late + PB, PB)], S_WO + 2)

    def scores(pair):
        slot = pair % 2
        wait_all(k_v.at[slot], S_K + slot)
        s = jnp.dot(q_v[pair], k_v[slot], preferred_element_type=F32) * DH ** -0.5
        e = jnp.exp(s - jnp.max(s, axis=-1, keepdims=True))
        p_v[...] = e.astype(BF16)
        return 1.0 / jnp.sum(e, axis=-1, keepdims=True)

    def values(pair):
        slot = pair % 2
        wait_all(v_v.at[slot], S_V + slot)
        return lax.dot_general(p_v[...], v_v[slot], nt, preferred_element_type=F32)

    def project(o, inv_l, pair):
        o = jnp.where(own, o * inv_l, 0.0).astype(BF16)
        r = None
        for i in range(PB):
            j = pair * PB + i
            t = jnp.dot(o[:, i * 128:(i + 1) * 128], wo_v[j // nblk, j % nblk],
                        preferred_element_type=F32)
            r = t if r is None else r + t
        return r

    def stage(s, acc):
        issue_kv(True, s)
        inv_l = scores(s)
        issue_kv(False, s + 1)
        return acc + project(values(s), inv_l, s)

    acc = lax.fori_loop(0, last - 1, stage, jnp.zeros((8, D), F32))

    issue_kv(True, last - 1)
    inv_l = scores(last - 1)
    issue(_merge([P(kv_piece, False, last, 0, cb) for cb in range(ncb)],
                 [P(last_v_piece, 1, cb) for cb in range(ncb)]))
    o = jnp.where(own, values(last - 1) * inv_l, 0.0)
    o = o + pltpu.roll(o, 1, 0)
    for i in range(PB):
        occ[i * 128:(i + 1) * 128, :] = column(o[0:1, i * 128:(i + 1) * 128])

    va = [P(last_v_piece, 0, cb) for cb in range(ncb)]
    lw = [P(late_wo_piece, r) for r in range(0, PAIR, 32)]
    k = ncb - 2 * MOVE
    tail = _merge(va[:k] + va[k::2] + lw[0::2],
                  va[k + 1::2] + lw[1::2] + [P(gate_piece, r) for r in range(0, D, 16)])
    issue(tail[:2 * FIFO])
    inv_l = scores(last)
    xc = x + ga * (acc + pltpu.roll(acc, 1, 0))
    shift = _mean(xc)
    xc = xc - shift

    vs = last % 2
    c0 = 0
    for ci, cw in enumerate(TAIL_V):
        wait_all(v_v.at[vs, :, pl.ds(c0, cw)], S_TV + ci)
        if ci == 0:
            issue(tail[2 * FIFO:])
        o = lax.dot_general(p_v[:, c0:c0 + cw], v_v[vs, :, c0:c0 + cw], nt,
                            preferred_element_type=F32)
        if ci > 0:
            o = o + o_v[...]
        if ci < len(TAIL_V) - 1:
            o_v[...] = o
        c0 += cw
    t = project(o, inv_l, last)
    xc = xc + ga * (t + pltpu.roll(t, 1, 0))

    def vpu_matvec(w, col, part=None):
        for r in range(0, w.shape[0], 16):
            prod = w[r:r + 16, :].astype(F32) * jnp.tile(col[r:r + 16, :], (1, nd))
            part = prod if part is None else part + prod
        return part

    part = None
    r0 = 0
    for ci, n in enumerate(TAIL_WO):
        rows = wo_v.at[WO_G - 1, b_late + r0 // 128, pl.ds(r0 % 128, n)]
        wait_all(rows, S_TO + ci)
        part = vpu_matvec(rows, occ.at[pl.ds(r0, n)], part)
        r0 += n
    xc = xc + ga * _sublane_allsum(part[:8] + part[8:])
    x1 = xc + shift

    xa = xc * A
    d1, e2 = _mean(xc), _mean(xc * xc)
    exa, exa2, exaa, exab = _mean(xa), _mean(xa * xa), _mean(xc * A2), _mean(xc * AB)
    r1 = lax.rsqrt(jnp.maximum(e2 - d1 * d1, 0.0) + EPS)
    mu = exa - d1 * eA
    p2 = exa2 - d1 * (2.0 * exaa - d1 * eA2) - mu * mu
    p1 = 2.0 * (exab - d1 * eAB)
    r2 = lax.rsqrt(jnp.maximum((p2 * r1 + p1) * r1 + eB2, 0.0) + EPS)
    hm = ((xa - d1 * A - mu) * r1 + Bc) * r2

    rowp = lax.broadcasted_iota(jnp.int32, (8, AT * 128), 0)
    h1 = hm[:, :AT * 128]
    h2 = h1 * h1
    groups = []
    for pw in (h1, h2, h2 * h1):
        ph, pm, pl_ = _split3(pw)
        groups.append(_rows(rowp, (ph, pm, ph, pl_, ph, pm, 1.0)))
    hp = jnp.concatenate(groups, axis=0)

    def mxu_arg(j):
        return jnp.concatenate([jnp.concatenate([
            jnp.dot(cz_v[r:r + SPLIT, :], hp[:, t * 128:(t + 1) * 128], preferred_element_type=F32)
            for r in range(j * BLK, (j + 1) * BLK, SPLIT)], axis=0) for t in range(AT)], axis=1)

    def tanh_rows(h, r, n, z_mxu):
        k = 0 if z_mxu is None else AT
        s = (jnp.tile(h[:, k * 128:], (n // 8, 1)) * jnp.tile(w1c[r:r + n, :], (1, nd - k))
             + jnp.tile(b1c[r:r + n, :], (1, nd - k)))
        z = s * (s * s + GELU_K)
        return jnp.tanh(z if z_mxu is None else jnp.concatenate([z_mxu, z], axis=1))

    nb = F // BLK
    acc_r = [lin]
    ahead = {j: mxu_arg(j) for j in range(FIRST, LOOK)}
    for j in range(nb - CARRY):
        if j + LOOK < nb:
            ahead[j + LOOK] = mxu_arg(j + LOOK)
        th = tanh_rows(hm, j * BLK, BLK, ahead.pop(j, None))
        acc_r.append(acc_r[-1] + jnp.dot(lhs_v[j], th, preferred_element_type=F32))
    hd = hm + jnp.tile(0.0 * acc_r[-3][:, 128:256], (1, nd))
    for i in range(CARRY):
        j = nb - CARRY + i
        z_mxu = ahead.pop(j)
        for r in range(0, BLK, 8):
            th_v[i, r:r + 8, :] = tanh_rows(hd, j * BLK + r, 8, z_mxu[r:r + 8])

    part = None
    r0 = 0
    for ci, n in enumerate(TAIL_GATE):
        rows = gb_v.at[pl.ds(r0, n)]
        wait_all(rows, S_GB + ci)
        if ci == 0:
            R = acc_r[-1]
            for i in range(CARRY):
                R = R + jnp.dot(lhs_v[nb - CARRY + i], th_v[i], preferred_element_type=F32)
            R = R + pltpu.roll(R, 7, 0)
            y = hm * R + pltpu.roll(R, 4, 0)
        part = vpu_matvec(rows, scc.at[pl.ds(r0, n)], part)
        r0 += n
    gb = _sublane_allsum(part[:8] + part[8:])
    o_ref[...] = (x1 + gb * y)[0:1].astype(o_ref.dtype)


@jax.jit
def pallas_adaLN_cond__sliding_block_cached__mixer_token_mlp__decode_kernel(
    A_x: jax.Array,
    A_k_cache: jax.Array,
    A_v_cache: jax.Array,
    A_wq: jax.Array,
    A_wo: jax.Array,
    B_x: jax.Array,
    B_w1: jax.Array,
    B_b1: jax.Array,
    B_w2: jax.Array,
    B_b2: jax.Array,
    c: jax.Array,
    w_mod: jax.Array,
):
    B, SQ, D = A_x.shape
    _, HKV, SK, dh = A_k_cache.shape
    S, F = B_w1.shape
    assert B == 1 and SQ == 1 and S == 1 and HKV == HQ and dh == DH
    W = min(4096, max(256, SK // 4))
    assert sum(TAIL_V) == W and sum(TAIL_WO) == PAIR and sum(TAIL_GATE) == D
    NQ = HQ * DH

    kt = jnp.swapaxes(A_k_cache, 2, 3).reshape(NPAIR, PAIR, SK)
    vt = jnp.swapaxes(A_v_cache, 2, 3).reshape(NPAIR, PAIR, SK)
    args = (
        A_x.reshape(1, D), kt, vt, A_wq.reshape(WQ_G, D // WQ_G, NQ),
        A_wo.reshape(WO_G, NQ // WO_G // 128, 128, D),
        B_w1, B_b1.reshape(F // 128, 128), B_w2.reshape(1, F), B_b2.reshape(1, 1),
        c, w_mod.reshape(WM_G, D // WM_G, 6 * D), w_mod,
    )
    out = pl.pallas_call(
        functools.partial(_kernel, D=D, F=F, SK=SK, W=W),
        out_shape=jax.ShapeDtypeStruct((1, D), A_x.dtype),
        in_specs=[pl.BlockSpec(memory_space=pl.ANY)] * len(args),
        out_specs=pl.BlockSpec(memory_space=pltpu.VMEM),
        scratch_shapes=[
            pltpu.VMEM((1, D), BF16),
            pltpu.VMEM((1, D), BF16),
            pltpu.VMEM((1, F), BF16),
            pltpu.VMEM((F // 128, 128), BF16),
            pltpu.VMEM((1, F), BF16),
            pltpu.VMEM((1, 1), BF16),
            pltpu.VMEM((WM_G, D // WM_G, 5 * D), BF16),
            pltpu.VMEM((D, D), BF16),
            pltpu.VMEM((WQ_G, D // WQ_G, NQ), BF16),
            pltpu.VMEM((WO_G, NQ // WO_G // 128, 128, D), BF16),
            pltpu.VMEM((2, PAIR, W), BF16),
            pltpu.VMEM((2, PAIR, W), BF16),
            pltpu.VMEM((NPAIR, 8, PAIR), BF16),
            pltpu.VMEM((8, W), BF16),
            pltpu.VMEM((8, PAIR), F32),
            pltpu.VMEM((CARRY, BLK, D), F32),
            pltpu.VMEM((F, 128), F32),
            pltpu.VMEM((F, 128), F32),
            pltpu.VMEM((F, 24), F32),
            pltpu.VMEM((D, 128), F32),
            pltpu.VMEM((PAIR, 128), F32),
            pltpu.VMEM((F // BLK, 8, BLK), F32),
            pltpu.SemaphoreType.DMA((N_SEMS,)),
        ],
        compiler_params=pltpu.CompilerParams(
            vmem_limit_bytes=64 * 1024 * 1024,
            disable_bounds_checks=True,
            disable_semaphore_checks=True,
        ),
    )(*args)
    return out.reshape(B, SQ, D)
```

```python
import functools
import math

import jax
import jax.numpy as jnp
from jax import lax
import jax.experimental.pallas as pl
import jax.experimental.pallas.tpu as pltpu

F32 = jnp.float32
BF16 = jnp.bfloat16

HQ = 32
DH = 192
PAIR = 2 * DH
NPAIR = HQ // 2
PB = PAIR // 128
EPS = 1e-5
GELU_C = math.sqrt(2.0 / math.pi)
GELU_A = 0.044715
GELU_S = (GELU_C * GELU_A) ** (1.0 / 3.0)
GELU_K = GELU_C / GELU_S

LEAD = 26
FIFO = 28
WM_G = 4
SEG = 256
GROUPS = ((0, 192, 32), (224, 136, 24))
LAST_GROUPS = ((0, 224, 32), (256, 112, 16))
TAIL_V = ((2048, 2048), (2048, 1536, 512))
XB, XA = 24, 8
CUTS = (28, 44, 60, 76)
TAIL_WO = (128, 128, 64, 64)
TAIL_GATE = (448, 96, 64, 32)
BLK = 96
AT = 2
FIRST, LOOK = 2, 3
SPLIT = 48
CARRY = 2

S_SMALL, S_WM, S_WQ = 0, 1, 2
S_WO = 3
S_K, S_V = 5, 6
S_TV = 7
S_TO = S_TV + sum(len(t) for t in TAIL_V)
S_GB = S_TO + len(TAIL_WO)
N_SEMS = S_GB + len(TAIL_GATE)


def _mean(t):
    return jnp.mean(t, axis=-1, keepdims=True)


def _chunk_of(pos, chunks):
    end = 0
    for ci, n in enumerate(chunks):
        end += n
        if pos < end:
            return ci
    raise ValueError(pos)


def _sublane_allsum(t):
    t = t + pltpu.roll(t, 4, 0)
    t = t + pltpu.roll(t, 2, 0)
    return t + pltpu.roll(t, 1, 0)


def _split3(t):
    hi = t.astype(BF16).astype(F32)
    r = t - hi
    mid = r.astype(BF16).astype(F32)
    return hi, mid, (r - mid).astype(BF16).astype(F32)


def _rows(row, vals):
    out = jnp.zeros(row.shape, F32)
    done = []
    for v in vals:
        if any(v is d for d in done):
            continue
        done.append(v)
        m = None
        for i, u in enumerate(vals):
            if u is v:
                m = (row == i) if m is None else m | (row == i)
        out = jnp.where(m, v, out)
    return out


def _merge(a, b):
    out = []
    for i in range(max(len(a), len(b))):
        if i < len(a):
            out.append((a[i], 0))
        if i < len(b):
            out.append((b[i], 1))
    return out


def _kernel(x_hbm, k_hbm, v_hbm, wq_hbm, wo_hbm, wo2_hbm, w1_hbm, b1_hbm, w2_hbm, b2_hbm,
            c_hbm, wm_hbm, wm2_hbm, o_ref,
            x_v, c_v, w1_v, b1_v, w2_v, b2_v, wm_v, gb_v, wq_v, wo_v, lw_v, k_v, v_v,
            q_v, p_v, oa_v, o_v, th_v, w1c, b1c, cz_v, scc, occ, lhs_v, sems, *, D, F, SK, W):
    col0 = SK - W
    ncb = W // 128
    NQ = HQ * DH
    nd = D // 128
    late, last = NPAIR - 1, NPAIR - 2
    nseg = wq_v.shape[0]
    t_late = SEG - PAIR // 8 * nd
    P = functools.partial

    def wait_all(buf, sem):
        pltpu.make_async_copy(buf, buf, sems.at[sem]).wait()

    def kv_piece(seg, is_b, cb):
        is_v, pair, g = seg
        src, dst, sem = (v_hbm, v_v, S_V) if is_v else (k_hbm, k_v, S_K)
        r0, nb_, na = GROUPS[g]
        if is_v and isinstance(pair, int) and pair == last:
            r0, nb_, na = LAST_GROUPS[g]
            sem = S_TV + sum(len(t) for t in TAIL_V[:g]) + _chunk_of(cb * 128, TAIL_V[g])
        rows = pl.ds(r0, nb_) if is_b else pl.ds(r0 + nb_, na)
        c = cb * 128
        if not isinstance(cb, int):
            c = pl.multiple_of(c, 128)
        return pltpu.make_async_copy(
            src.at[pair, rows, pl.ds(col0 + c, 128)], dst.at[rows, pl.ds(c, 128)], sems.at[sem])

    def seg_list(seg, is_b):
        return [P(kv_piece, seg, is_b, cb) for cb in range(ncb)]

    def wm_piece(r, sec):
        idx = (slice(None), pl.ds(r, 8), pl.ds(sec * D, D))
        return pltpu.make_async_copy(wm_hbm.at[idx], wm_v.at[idx], sems.at[S_WM])

    def wq_piece(t):
        return pltpu.make_async_copy(wq_hbm.at[:, t], wq_v.at[:, t], sems.at[S_WQ])

    def wo_piece(t):
        idx = (pl.ds(0, nseg - (t >= t_late)), t)
        return pltpu.make_async_copy(wo_hbm.at[idx], wo_v.at[idx], sems.at[S_WO + (t >= t_late)])

    def late_wo_piece(r, n):
        return pltpu.make_async_copy(wo2_hbm.at[pl.ds(late * PAIR + r, n), :], lw_v.at[pl.ds(r, n), :],
                                     sems.at[S_TO + _chunk_of(r, TAIL_WO)])

    def from_tiles(ref, ntile, i0, ni, j0, nj):
        return jnp.concatenate([jnp.concatenate(
            [ref[divmod(i * ntile + j, SEG)].astype(F32) for j in range(j0, j0 + nj)], axis=1)
            for i in range(i0, i0 + ni)], axis=0)

    def gate_piece(r):
        return pltpu.make_async_copy(
            wm2_hbm.at[pl.ds(r, 16), pl.ds(5 * D, D)], gb_v.at[pl.ds(r, 16), :],
            sems.at[S_GB + _chunk_of(r, TAIL_GATE)])

    def issue(lst):
        for f, prio in lst:
            f().start(priority=prio)

    def issue_seg(seg, nxt):
        def same(cb, carry):
            kv_piece(seg, False, cb).start(priority=0)
            kv_piece(seg, True, cb + LEAD).start(priority=1)
            return carry

        def ahead(cb, carry):
            kv_piece(seg, False, cb + ncb - LEAD).start(priority=0)
            kv_piece(nxt, True, cb).start(priority=1)
            return carry
        lax.fori_loop(0, ncb - LEAD, same, 0, unroll=2)
        lax.fori_loop(0, LEAD, ahead, 0, unroll=2)

    def issue_kv(is_v, pair, after=None):
        nxt = (False, after) if is_v else (True, pair)
        issue_seg((is_v, pair, 1), nxt + (0,))
        issue_seg(nxt + (0,), nxt + (1,))

    wm_p = [P(wm_piece, r, s) for r in range(0, D // WM_G, 8) for s in range(5)]
    seq_a = wm_p[:len(wm_p) // 2] + [P(wo_piece, t) for t in range(SEG)]
    seq_b = (wm_p[len(wm_p) // 2:] + [P(wq_piece, t) for t in range(SEG)]
             + seg_list((False, 0, 0), True)[:LEAD])
    head = [(f, 1) for f in seq_b[:LEAD]] + _merge(seq_a, seq_b[LEAD:])
    cut1 = LEAD + len(wm_p) + 2 * FIFO

    small = [pltpu.make_async_copy(src, dst, sems.at[S_SMALL]) for src, dst in (
        (x_hbm, x_v), (c_hbm, c_v), (w1_hbm, w1_v), (b1_hbm, b1_v), (w2_hbm, w2_v),
        (b2_hbm, b2_v))]
    for cp in small:
        cp.start()
    issue(head[:cut1])
    for cp in small:
        cp.wait()
    wait_all(wm_v, S_WM)

    x = jnp.broadcast_to(x_v[...].astype(F32), (8, D))
    cc = c_v[...].astype(F32)
    sc = (cc * jax.nn.sigmoid(cc)).astype(BF16).astype(F32)
    sc8 = jnp.broadcast_to(sc, (8, D)).astype(BF16)
    mod = jnp.dot(sc8, wm_v[...].reshape(D, 5 * D), preferred_element_type=F32)
    sa, ca, ga, sb, cb_ = (mod[:, i * D:(i + 1) * D] for i in range(5))
    xm = x - _mean(x)
    h8 = (xm * lax.rsqrt(_mean(xm * xm) + EPS) * (1.0 + ca) + sa).astype(BF16).astype(F32)
    A = 1.0 + cb_
    Bc = sb - _mean(sb)
    A2, AB = A * A, A * Bc
    eA, eA2, eAB, eB2 = _mean(A), _mean(A2), _mean(AB), _mean(Bc * Bc)

    eye = (lax.broadcasted_iota(jnp.int32, (128, 128), 0)
           == lax.broadcasted_iota(jnp.int32, (128, 128), 1))
    ones = jnp.ones((128, 128), BF16)
    ident = jnp.where(eye, 1.0, 0.0)
    nt = (((1,), (1,)), ((), ()))

    def column(rowvec):
        diag = jnp.where(eye, jnp.broadcast_to(rowvec, (128, 128)), 0.0).astype(BF16)
        return jnp.dot(diag, ones, preferred_element_type=F32)

    for r in range(0, D, 128):
        scc[r:r + 128, :] = column(sc[:, r:r + 128])

    w1r = w1_v[...].astype(F32)
    w2r = w2_v[...].astype(F32)
    b1r = b1_v[...].astype(F32)
    row128 = lax.broadcasted_iota(jnp.int32, (8, 128), 0)
    lin = jnp.zeros((8, 128), F32)
    lhs = []
    for j in range(F // 128):
        sl = slice(j * 128, (j + 1) * 128)
        r1, rb, r2 = w1r[:, sl], b1r[j:j + 1, :], w2r[:, sl]
        w1c[sl, :] = column(r1) * GELU_S
        b1c[sl, :] = column(rb) * GELU_S
        t = jnp.where(row128 < 4, r1, rb) * (0.5 * r2)
        hi = t.astype(BF16).astype(F32)
        lo = (t - hi).astype(BF16).astype(F32)
        lhs.append(jnp.where(row128 % 4 == 0, hi, jnp.where(row128 % 4 == 1, lo, 0.0)))
        lin = lin + t
        w, b = r1 * GELU_S, rb * GELU_S
        c0 = _split3(b * (b * b + GELU_K))
        groups = []
        for i, cf in enumerate((w * (3.0 * b * b + GELU_K), 3.0 * w * w * b, w * w * w)):
            ch, cm, cl = _split3(cf)
            groups.append(_rows(row128, (ch, ch, cm, ch, cl, cm, c0[i])))
        cz_v[sl, :] = lax.dot_general(ident, jnp.concatenate(groups, axis=0), nt,
                                      preferred_element_type=F32)
    lhs = jnp.concatenate(lhs, axis=1)
    for j in range(F // BLK):
        lhs_v[j] = lhs[:, j * BLK:(j + 1) * BLK]
    lin = jnp.sum(lin, axis=-1, keepdims=True)
    lin = lin + jnp.where(lax.broadcasted_iota(jnp.int32, (8, 1), 0) < 4, 0.0,
                          b2_v[...].astype(F32))
    lin = jnp.where(lax.broadcasted_iota(jnp.int32, (8, D), 0) % 4 == 0,
                    jnp.broadcast_to(lin, (8, D)), 0.0)

    issue(head[cut1:])
    issue_seg((False, 0, 0), (False, 0, 1))
    wait_all(wq_v, S_WQ)
    wait_all(wo_v.at[:, pl.ds(0, t_late)], S_WO)
    wait_all(wo_v.at[pl.ds(0, nseg - 1), pl.ds(t_late, SEG - t_late)], S_WO + 1)
    own = ((lax.broadcasted_iota(jnp.int32, (8, PAIR), 1) >= DH)
           == (lax.broadcasted_iota(jnp.int32, (8, PAIR), 0) % 2 == 1))
    for p in range(NPAIR):
        q = jnp.dot(h8, from_tiles(wq_v, NQ // 128, 0, D // 8, p * PB, PB),
                    preferred_element_type=F32)
        q_v[p] = jnp.where(own, q, 0.0).astype(BF16)

    def scores(pair):
        wait_all(k_v, S_K)
        s = jnp.dot(q_v[pair], k_v[...], preferred_element_type=F32) * DH ** -0.5
        e = jnp.exp(s - jnp.max(s, axis=-1, keepdims=True))
        p_v[...] = e.astype(BF16)
        return 1.0 / jnp.sum(e, axis=-1, keepdims=True)

    def values(pair):
        wait_all(v_v, S_V)
        return lax.dot_general(p_v[...], v_v[...], nt, preferred_element_type=F32)

    def normalise(o, inv_l, mask):
        return jnp.where(mask, o * inv_l, 0.0).astype(BF16).astype(F32)

    def project(o, r0):
        return jnp.dot(o, from_tiles(wo_v, nd, r0 // 8, o.shape[1] // 8, 0, nd),
                       preferred_element_type=F32)

    def stage(s, carry):
        issue_kv(False, s)
        inv_l = scores(s)
        issue_kv(True, s, jnp.where(s + 1 == last, late, s + 1))
        oa_v[s] = normalise(values(s), inv_l, own)
        return carry

    lax.fori_loop(0, last, stage, 0)

    issue_seg((False, late, 1), (True, late, 0))
    acc = project(oa_v[0], 0)
    for p in range(1, last):
        acc = acc + project(oa_v[p], p * PAIR)
    issue_seg((True, late, 0), (True, late, 1))
    inv_l = scores(late)
    issue_kv(True, late, last)
    o = normalise(values(late), inv_l, own)
    o = o + pltpu.roll(o, 1, 0)
    for i in range(PB):
        occ[i * 128:(i + 1) * 128, :] = column(o[0:1, i * 128:(i + 1) * 128])

    segs = ((False, last, 1), (True, last, 0), (True, last, 1))
    xs = range(0, PAIR, XB + XA)
    ta = [f for g in segs for f in seg_list(g, False)] + [P(late_wo_piece, r + XB, XA) for r in xs]
    tb = ([f for g in segs for f in seg_list(g, True)] + [P(late_wo_piece, r, XB) for r in xs]
          + [P(gate_piece, r) for r in range(0, D, 16)])
    tail = _merge(ta, tb[LEAD:])
    cuts = [0] + [2 * (ncb + c) for c in CUTS] + [len(tail)] * 2
    issue(tail[:cuts[1]])
    inv_l = scores(last)
    xc = x + ga * (acc + pltpu.roll(acc, 1, 0))
    shift = _mean(xc)
    xc = xc - shift

    ci = 0
    for g, (r0, nb_, na) in enumerate(LAST_GROUPS):
        r1 = r0 + nb_ + na
        c0 = 0
        for k, cw in enumerate(TAIL_V[g]):
            wait_all(v_v.at[r0:r1, pl.ds(c0, cw)], S_TV + ci)
            issue(tail[cuts[ci + 1]:cuts[ci + 2]])
            o = lax.dot_general(p_v[:, c0:c0 + cw], v_v[r0:r1, c0:c0 + cw], nt,
                                preferred_element_type=F32)
            if k > 0:
                o = o + o_v[:, r0:r1]
            if k < len(TAIL_V[g]) - 1:
                o_v[:, r0:r1] = o
            c0 += cw
            ci += 1
        t = project(normalise(o, inv_l, own[:, r0:r1]), last * PAIR + r0)
        xc = xc + ga * (t + pltpu.roll(t, 1, 0))

    def vpu_matvec(w, col, part=None):
        for r in range(0, w.shape[0], 16):
            prod = w[r:r + 16, :].astype(F32) * jnp.tile(col[r:r + 16, :], (1, nd))
            part = prod if part is None else part + prod
        return part

    part = None
    r0 = 0
    for ci, n in enumerate(TAIL_WO):
        rows = lw_v.at[pl.ds(r0, n)]
        wait_all(rows, S_TO + ci)
        part = vpu_matvec(rows, occ.at[pl.ds(r0, n)], part)
        r0 += n
    xc = xc + ga * _sublane_allsum(part[:8] + part[8:])
    x1 = xc + shift

    xa = xc * A
    d1, e2 = _mean(xc), _mean(xc * xc)
    exa, exa2, exaa, exab = _mean(xa), _mean(xa * xa), _mean(xc * A2), _mean(xc * AB)
    r1 = lax.rsqrt(jnp.maximum(e2 - d1 * d1, 0.0) + EPS)
    mu = exa - d1 * eA
    p2 = exa2 - d1 * (2.0 * exaa - d1 * eA2) - mu * mu
    p1 = 2.0 * (exab - d1 * eAB)
    r2 = lax.rsqrt(jnp.maximum((p2 * r1 + p1) * r1 + eB2, 0.0) + EPS)
    hm = ((xa - d1 * A - mu) * r1 + Bc) * r2

    rowp = lax.broadcasted_iota(jnp.int32, (8, AT * 128), 0)
    h1 = hm[:, :AT * 128]
    h2 = h1 * h1
    groups = []
    for pw in (h1, h2, h2 * h1):
        ph, pm, pl_ = _split3(pw)
        groups.append(_rows(rowp, (ph, pm, ph, pl_, ph, pm, 1.0)))
    hp = jnp.concatenate(groups, axis=0)

    def mxu_arg(j):
        return jnp.concatenate([jnp.concatenate([
            jnp.dot(cz_v[r:r + SPLIT, :], hp[:, t * 128:(t + 1) * 128], preferred_element_type=F32)
            for r in range(j * BLK, (j + 1) * BLK, SPLIT)], axis=0) for t in range(AT)], axis=1)

    def tanh_rows(h, r, n, z_mxu):
        k = 0 if z_mxu is None else AT
        s = (jnp.tile(h[:, k * 128:], (n // 8, 1)) * jnp.tile(w1c[r:r + n, :], (1, nd - k))
             + jnp.tile(b1c[r:r + n, :], (1, nd - k)))
        z = s * (s * s + GELU_K)
        return jnp.tanh(z if z_mxu is None else jnp.concatenate([z_mxu, z], axis=1))

    nb = F // BLK
    acc_r = [lin]
    ahead = {j: mxu_arg(j) for j in range(FIRST, LOOK)}
    for j in range(nb - CARRY):
        if j + LOOK < nb:
            ahead[j + LOOK] = mxu_arg(j + LOOK)
        th = tanh_rows(hm, j * BLK, BLK, ahead.pop(j, None))
        acc_r.append(acc_r[-1] + jnp.dot(lhs_v[j], th, preferred_element_type=F32))
    hd = hm + jnp.tile(0.0 * acc_r[-3][:, :128], (1, nd))
    for i in range(CARRY):
        j = nb - CARRY + i
        z_mxu = ahead.pop(j)
        for r in range(0, BLK, 8):
            th_v[i, r:r + 8, :] = tanh_rows(hd, j * BLK + r, 8, z_mxu[r:r + 8])

    part = None
    r0 = 0
    for ci, n in enumerate(TAIL_GATE):
        rows = gb_v.at[pl.ds(r0, n)]
        wait_all(rows, S_GB + ci)
        if ci == 0:
            R = acc_r[-1]
            for i in range(CARRY):
                R = R + jnp.dot(lhs_v[nb - CARRY + i], th_v[i], preferred_element_type=F32)
            R = R + pltpu.roll(R, 7, 0)
            y = hm * R + pltpu.roll(R, 4, 0)
        part = vpu_matvec(rows, scc.at[pl.ds(r0, n)], part)
        r0 += n
    gb = _sublane_allsum(part[:8] + part[8:])
    o_ref[...] = (x1 + gb * y)[0:1].astype(o_ref.dtype)


@jax.jit
def pallas_adaLN_cond__sliding_block_cached__mixer_token_mlp__decode_kernel(
    A_x: jax.Array,
    A_k_cache: jax.Array,
    A_v_cache: jax.Array,
    A_wq: jax.Array,
    A_wo: jax.Array,
    B_x: jax.Array,
    B_w1: jax.Array,
    B_b1: jax.Array,
    B_w2: jax.Array,
    B_b2: jax.Array,
    c: jax.Array,
    w_mod: jax.Array,
):
    B, SQ, D = A_x.shape
    _, HKV, SK, dh = A_k_cache.shape
    S, F = B_w1.shape
    assert B == 1 and SQ == 1 and S == 1 and HKV == HQ and dh == DH
    W = min(4096, max(256, SK // 4))
    assert all(sum(t) == W for t in TAIL_V) and sum(TAIL_WO) == PAIR and sum(TAIL_GATE) == D
    NQ = HQ * DH

    kt = jnp.swapaxes(A_k_cache, 2, 3).reshape(NPAIR, PAIR, SK)
    vt = jnp.swapaxes(A_v_cache, 2, 3).reshape(NPAIR, PAIR, SK)

    def tiles(w):
        r, n = w.shape
        return w.reshape(r // 8, 8, n // 128, 128).transpose(0, 2, 1, 3).reshape(-1, SEG, 8, 128)

    args = (
        A_x.reshape(1, D), kt, vt, tiles(A_wq), tiles(A_wo), A_wo,
        B_w1, B_b1.reshape(F // 128, 128), B_w2.reshape(1, F), B_b2.reshape(1, 1),
        c, w_mod.reshape(WM_G, D // WM_G, 6 * D), w_mod,
    )
    out = pl.pallas_call(
        functools.partial(_kernel, D=D, F=F, SK=SK, W=W),
        out_shape=jax.ShapeDtypeStruct((1, D), A_x.dtype),
        in_specs=[pl.BlockSpec(memory_space=pl.ANY)] * len(args),
        out_specs=pl.BlockSpec(memory_space=pltpu.VMEM),
        scratch_shapes=[
            pltpu.VMEM((1, D), BF16),
            pltpu.VMEM((1, D), BF16),
            pltpu.VMEM((1, F), BF16),
            pltpu.VMEM((F // 128, 128), BF16),
            pltpu.VMEM((1, F), BF16),
            pltpu.VMEM((1, 1), BF16),
            pltpu.VMEM((WM_G, D // WM_G, 5 * D), BF16),
            pltpu.VMEM((D, D), BF16),
            pltpu.VMEM((D * NQ // 1024 // SEG, SEG, 8, 128), BF16),
            pltpu.VMEM((D * NQ // 1024 // SEG, SEG, 8, 128), BF16),
            pltpu.VMEM((PAIR, D), BF16),
            pltpu.VMEM((PAIR, W), BF16),
            pltpu.VMEM((PAIR, W), BF16),
            pltpu.VMEM((NPAIR, 8, PAIR), BF16),
            pltpu.VMEM((8, W), BF16),
            pltpu.VMEM((NPAIR - 2, 8, PAIR), F32),
            pltpu.VMEM((8, PAIR), F32),
            pltpu.VMEM((CARRY, BLK, D), F32),
            pltpu.VMEM((F, 128), F32),
            pltpu.VMEM((F, 128), F32),
            pltpu.VMEM((F, 24), F32),
            pltpu.VMEM((D, 128), F32),
            pltpu.VMEM((PAIR, 128), F32),
            pltpu.VMEM((F // BLK, 8, BLK), F32),
            pltpu.SemaphoreType.DMA((N_SEMS,)),
        ],
        compiler_params=pltpu.CompilerParams(
            vmem_limit_bytes=64 * 1024 * 1024,
            disable_bounds_checks=True,
            disable_semaphore_checks=True,
        ),
    )(*args)
    return out.reshape(B, SQ, D)
```
